```python
import jax
import jax.numpy as jnp

def _softmax(x, axis=-1):
    return jax.nn.softmax(x, axis=axis)
def _gelu(x):
    return jax.nn.gelu(x, approximate=True)
def _silu(x):
    return jax.nn.silu(x)
def _sigmoid(x):
    return jax.nn.sigmoid(x)
def _layernorm(x, axis=-1, eps=1e-5):
    m = jnp.mean(x, axis=axis, keepdims=True)
    v = jnp.var(x, axis=axis, keepdims=True)
    return (x - m) / jnp.sqrt(v + eps)
def _scatter_add(tgt, idx, src, axis=0):
    return tgt.at[idx].add(src)
def _segment_sum(src, seg, n):
    return jax.ops.segment_sum(src, seg, n)
class _Rng:
    def __init__(self, key):
        self._k = key
    def _next(self):
        self._k, sub = jax.random.split(self._k)
        return sub
    def normal(self, shape):
        return jax.random.normal(self._next(), shape, dtype=jnp.bfloat16)
    def randint(self, lo, hi, shape):
        return jax.random.randint(self._next(), shape, lo, hi, dtype=jnp.int32)
    def uniform(self, shape, lo=0.0, hi=1.0):
        return jax.random.uniform(self._next(), shape, jnp.bfloat16, lo, hi)
    def permutation(self, n):
        return jax.random.permutation(self._next(), n)


kernel_name = 'interleave_layers__sliding_block_cached__moe_arch_mod__decode'

def setup_inputs():
    _rng = _Rng(jax.random.key(int.from_bytes(__import__("os").urandom(4), "little")))
    _w = (lambda a: (lambda t: t.astype(jnp.bfloat16) if jnp.issubdtype(t.dtype, jnp.floating) else t)(jnp.asarray(a)))
    def _A_setup():
        B, Sq, D = 4, 1, 640
        Hq, Hkv, Sk, Dh = 32, 32, 4096, 192
        assert Hq % Hkv == 0, (Hq, Hkv)
        return {
            "x": _w((lambda *s: _rng.normal(s) * 0.05)(B, Sq, D)),
            "k_cache": _w((lambda *s: _rng.normal(s) * 0.05)(B, Hkv, Sk, Dh)),
            "v_cache": _w((lambda *s: _rng.normal(s) * 0.05)(B, Hkv, Sk, Dh)),
            "wq": _w((lambda *s: _rng.normal(s) * 0.05)(D, Hq * Dh) * (D ** -0.5)),
            "wo": _w((lambda *s: _rng.normal(s) * 0.05)(Hq * Dh, D) * ((Hq * Dh) ** -0.5)),
        }
    _A_in = _A_setup()

    def _B_setup():
        B, S, D, F, C = 4, 1, 640, 1536, 1
        return {
            "x": _w((lambda *s: _rng.normal(s) * 0.05)(B, S, D)),
            "w_r": _w((lambda *s: _rng.normal(s) * 0.05)(D)),
            "w_gate": _w((lambda *s: _rng.normal(s) * 0.05)(D, F)),
            "w_up": _w((lambda *s: _rng.normal(s) * 0.05)(D, F)),
            "w_down": _w((lambda *s: _rng.normal(s) * 0.05)(F, D)),
        }
    _B_in = _B_setup()

    return {
        "A_x": _A_in["x"],
        "A_k_cache": _A_in["k_cache"],
        "A_v_cache": _A_in["v_cache"],
        "A_wq": _A_in["wq"],
        "A_wo": _A_in["wo"],
        "B_x": _B_in["x"],
        "B_w_r": _B_in["w_r"],
        "B_w_gate": _B_in["w_gate"],
        "B_w_up": _B_in["w_up"],
        "B_w_down": _B_in["w_down"],
    }

def reference(A_x, A_k_cache, A_v_cache, A_wq, A_wo, B_x, B_w_r, B_w_gate, B_w_up, B_w_down):
    def _A_ref(x, k_cache, v_cache, wq, wo):
        B, Sq, D = x.shape
        Hq, Dh = 32, 192
        Hkv, Sk = k_cache.shape[1], k_cache.shape[2]
        W = min(4096, max(256, Sk // 4))
        rep = Hq // Hkv
        q = (lambda x, *d: x.transpose(*d))((x @ wq).reshape(B, Sq, Hq, Dh), 0, 2, 1, 3)
        k = jnp.repeat(k_cache[:, :, Sk - W:, :], rep, axis=1)
        v = jnp.repeat(v_cache[:, :, Sk - W:, :], rep, axis=1)
        scores = jnp.einsum("bhqd,bhkd->bhqk", q, k) * (Dh ** -0.5)
        p = _softmax(scores, axis=-1)
        o = jnp.einsum("bhqk,bhkd->bhqd", p, v)
        return (lambda x, *d: x.transpose(*d))(o, 0, 2, 1, 3).reshape(B, Sq, Hq * Dh) @ wo

    def _B_ref(x, w_r, w_gate, w_up, w_down):
        B, S, D = x.shape
        C = 1
        r = x @ w_r
        idx = jnp.argsort(-r, axis=-1)[:, :C]
        idx_e = jnp.repeat(idx.reshape(B, C, 1), D, axis=2)
        x_sel = jnp.take_along_axis(x, idx_e, axis=1)
        g = _silu(x_sel @ w_gate)
        u = x_sel @ w_up
        y = (g * u) @ w_down
        r_sel = _sigmoid(jnp.take_along_axis(r, idx, axis=1))
        y = y * r_sel.reshape(B, C, 1)
        b_off = (jnp.arange(B) * S).reshape(B, 1)
        flat_idx = (idx + b_off).reshape(B * C)
        zero = (x * 0.0).reshape(B * S, D)
        upd = _scatter_add(zero, flat_idx, y.reshape(B * C, D), axis=0)
        return x + upd.reshape(B, S, D)

    x = A_x
    x = x + _A_ref(_layernorm(x, axis=-1), A_k_cache, A_v_cache, A_wq, A_wo)
    x = x + _B_ref(_layernorm(x, axis=-1), B_w_r, B_w_gate, B_w_up, B_w_down)
    x = x + _A_ref(_layernorm(x, axis=-1), A_k_cache, A_v_cache, A_wq, A_wo)
    x = x + _B_ref(_layernorm(x, axis=-1), B_w_r, B_w_gate, B_w_up, B_w_down)
    return x
```

```python
import jax
import jax.numpy as jnp
from jax.experimental import pallas as pl
from jax.experimental.pallas import tpu as pltpu

B, D, H, DH, SK, F = 4, 640, 32, 192, 4096, 1536
W = min(4096, max(256, SK // 4))
HG = 8
NG = H // HG
NJ = B * NG
GW = HG * DH
GW2 = GW // 2
DH2 = DH // 2
EPS = 1e-5
SCALE = DH ** -0.5
NCOL = 4
LOOKAHEAD = 2

f32, bf16, u32 = jnp.float32, jnp.bfloat16, jnp.uint32


def _ln(x):
    m = jnp.mean(x, axis=-1, keepdims=True)
    xc = x - m
    v = jnp.mean(xc * xc, axis=-1, keepdims=True)
    return xc / jnp.sqrt(v + EPS)


def _as_bf16(w):
    return pltpu.bitcast(w, bf16)


def _mm(a, w):
    return jnp.dot(a, w, preferred_element_type=f32)


def _kernel(x_hbm, wr_hbm, k_hbm, v_hbm, wq_hbm, wo_hbm, wg_hbm, wu_hbm, wd_hbm,
            o_ref,
            kbuf, vbuf, wq_s, wo_s, wg_s, wu_s, wd_s, x_s, wr_s,
            ksem, vsem, wsem):
    k32, v32 = k_hbm.bitcast(u32), v_hbm.bitcast(u32)
    wq32, wo32 = wq_hbm.bitcast(u32), wo_hbm.bitcast(u32)
    wg32, wu32, wd32 = wg_hbm.bitcast(u32), wu_hbm.bitcast(u32), wd_hbm.bitcast(u32)
    cw = W // NCOL

    def start_kv(src, dst, sems, j):
        b = j // NG
        g = j % NG

        def head(i, carry):
            for c in range(NCOL):
                pltpu.make_async_copy(
                    src.at[b, g * HG + i, :, pl.ds(SK - W + c * cw, cw)],
                    dst.at[j, pl.ds(pl.multiple_of(i * DH2, 8), DH2), pl.ds(c * cw, cw)],
                    sems.at[j]).start(priority=c % 2)
            return carry

        jax.lax.fori_loop(0, HG, head, 0)

    def start_group(j):
        start_kv(k32, kbuf, ksem, j)
        start_kv(v32, vbuf, vsem, j)

    def wait_all(buf, sem):
        pltpu.make_async_copy(buf, buf, sem).wait()

    S_X, S_WR, S_WQ, S_WO, S_WG, S_WU, S_WD = range(7)

    def start_cols(src, dst, sem, ncols, piece):
        for c in range(ncols // piece):
            pltpu.make_async_copy(src.at[:, pl.ds(c * piece, piece)],
                                  dst.at[:, pl.ds(c * piece, piece)],
                                  sem).start(priority=c % 2)

    def start_rows(src, dst, sem, nrows, piece):
        for c in range(nrows // piece):
            pltpu.make_async_copy(src.at[pl.ds(c * piece, piece), :],
                                  dst.at[pl.ds(c * piece, piece), :],
                                  sem).start(priority=c % 2)

    for g in range(NG):
        start_cols(wq32.at[:, pl.ds(g * GW, GW)], wq_s.at[g], wsem.at[S_WQ], GW, 256)
    pltpu.make_async_copy(x_hbm, x_s, wsem.at[S_X]).start()
    pltpu.make_async_copy(wr_hbm, wr_s, wsem.at[S_WR]).start()
    start_group(0)
    start_rows(wo32, wo_s, wsem.at[S_WO], NG * GW2, 96)
    for j in range(1, LOOKAHEAD):
        start_group(j)

    wait_all(x_s, wsem.at[S_X])
    wait_all(wr_s, wsem.at[S_WR])
    x_all = x_s[...].astype(f32)
    wr = wr_s[...].astype(f32)
    wr_row = jnp.concatenate([wr[i:i + 1, :] for i in range(D // 128)], axis=1)
    wait_all(wq_s, wsem.at[S_WQ])

    row = jax.lax.broadcasted_iota(jnp.int32, (HG, GW), 0)
    col = jax.lax.broadcasted_iota(jnp.int32, (HG, GW), 1)
    mask = (col >= row * DH) & (col < row * DH + DH)
    row4 = jax.lax.broadcasted_iota(jnp.int32, (B, D), 0)

    def attention(x, b, first):
        h = _ln(x).astype(bf16)

        def group(g, acc):
            j = b * NG + g
            q = _mm(h, _as_bf16(wq_s[g]))
            qbd = jnp.where(mask, q, 0.0).astype(bf16)
            if first:
                wait_all(kbuf.at[j], ksem.at[j])
            s = _mm(qbd, _as_bf16(kbuf[j])) * SCALE
            m = jnp.max(s, axis=-1, keepdims=True)
            p = jnp.exp(s - m)
            l = jnp.sum(p, axis=-1, keepdims=True)
            if first:
                wait_all(vbuf.at[j], vsem.at[j])
            o = jax.lax.dot_general(p.astype(bf16), _as_bf16(vbuf[j]),
                                    (((1,), (1,)), ((), ())), preferred_element_type=f32)
            om = jnp.where(mask, o / l, 0.0).astype(bf16)
            if first:
                @pl.when(j == 0)
                def _():
                    wait_all(wo_s, wsem.at[S_WO])
            acc = acc + _mm(om, _as_bf16(wo_s[pl.ds(pl.multiple_of(g * GW2, 8), GW2), :]))
            if first:
                @pl.when(j + LOOKAHEAD < NJ)
                def _():
                    start_group(j + LOOKAHEAD)

                @pl.when(j == 0)
                def _():
                    start_cols(wg32, wg_s, wsem.at[S_WG], F, 256)
                    start_cols(wu32, wu_s, wsem.at[S_WU], F, 256)

                @pl.when(j == 1)
                def _():
                    start_rows(wd32, wd_s, wsem.at[S_WD], F // 2, 96)
            return acc

        acc = jax.lax.fori_loop(0, NG, group, jnp.zeros((HG, D), f32))
        return x + jnp.broadcast_to(jnp.sum(acc, axis=0, keepdims=True), (HG, D))

    def ffn(x):
        h = _ln(x)
        r = jnp.sum(h * wr_row, axis=-1, keepdims=True)
        hb = h.astype(bf16)
        g = _mm(hb, _as_bf16(wg_s[...]))
        u = _mm(hb, _as_bf16(wu_s[...]))
        a = (g * jax.nn.sigmoid(g) * u).astype(bf16)
        y = _mm(a, _as_bf16(wd_s[...]))
        return x + h + y * jax.nn.sigmoid(r)

    def batch(b, out):
        xb = jnp.sum(jnp.where(row4 == b, x_all, 0.0), axis=0, keepdims=True)
        x = jnp.broadcast_to(xb, (HG, D))
        x = attention(x, b, True)

        @pl.when(b == 0)
        def _():
            wait_all(wg_s, wsem.at[S_WG])
            wait_all(wu_s, wsem.at[S_WU])
            wait_all(wd_s, wsem.at[S_WD])

        x = ffn(x)
        x = attention(x, b, False)
        x = ffn(x)
        return jnp.where(row4 == b, x[:B, :], out)

    out = jax.lax.fori_loop(0, B, batch, jnp.zeros((B, D), f32))
    o_ref[...] = out.astype(o_ref.dtype)


@jax.jit
def pallas_interleave_layers__sliding_block_cached__moe_arch_mod__decode_kernel(
    A_x: jax.Array,
    A_k_cache: jax.Array,
    A_v_cache: jax.Array,
    A_wq: jax.Array,
    A_wo: jax.Array,
    B_x: jax.Array,
    B_w_r: jax.Array,
    B_w_gate: jax.Array,
    B_w_up: jax.Array,
    B_w_down: jax.Array,
):
    del B_x
    k_t = jnp.transpose(A_k_cache, (0, 1, 3, 2))
    v_t = jnp.transpose(A_v_cache, (0, 1, 3, 2))
    any_spec = pl.BlockSpec(memory_space=pl.ANY)
    out = pl.pallas_call(
        _kernel,
        out_shape=jax.ShapeDtypeStruct((B, D), A_x.dtype),
        in_specs=[any_spec] * 9,
        out_specs=pl.BlockSpec(memory_space=pltpu.VMEM),
        scratch_shapes=[
            pltpu.VMEM((NJ, GW2, W), u32),
            pltpu.VMEM((NJ, GW2, W), u32),
            pltpu.VMEM((NG, D // 2, GW), u32),
            pltpu.VMEM((NG * GW2, D), u32),
            pltpu.VMEM((D // 2, F), u32),
            pltpu.VMEM((D // 2, F), u32),
            pltpu.VMEM((F // 2, D), u32),
            pltpu.VMEM((B, D), bf16),
            pltpu.VMEM((D // 128, 128), bf16),
            pltpu.SemaphoreType.DMA((NJ,)),
            pltpu.SemaphoreType.DMA((NJ,)),
            pltpu.SemaphoreType.DMA((8,)),
        ],
        compiler_params=pltpu.CompilerParams(vmem_limit_bytes=126 * 1024 * 1024),
    )(A_x.reshape(B, D), B_w_r.reshape(D // 128, 128), k_t, v_t,
      A_wq, A_wo, B_w_gate, B_w_up, B_w_down)
    return out.reshape(B, 1, D)
```

```python
import jax
import jax.numpy as jnp
from jax.experimental import pallas as pl
from jax.experimental.pallas import tpu as pltpu

B, D, H, DH, SK, F = 4, 640, 32, 192, 4096, 1536
W = min(4096, max(256, SK // 4))
HG = 8
NG = H // HG
NJ = B * NG
GW = HG * DH
GW2 = GW // 2
DH2 = DH // 2
EPS = 1e-5
SCALE = DH ** -0.5
NCOL = 4
QLEAD = 2
WLAG = 48

f32, bf16, u32 = jnp.float32, jnp.bfloat16, jnp.uint32


def _ln(x):
    m = jnp.mean(x, axis=-1, keepdims=True)
    xc = x - m
    v = jnp.mean(xc * xc, axis=-1, keepdims=True)
    return xc / jnp.sqrt(v + EPS)


def _as_bf16(w):
    return pltpu.bitcast(w, bf16)


def _mm(a, w):
    return jnp.dot(a, w, preferred_element_type=f32)


def _kernel(x_hbm, wr_hbm, k_hbm, v_hbm, wq_hbm, wo_hbm, wg_hbm, wu_hbm, wd_hbm,
            o_ref,
            kbuf, vbuf, wq_s, wo_s, wg_s, wu_s, wd_s, x_s, wr_s,
            ksem, vsem, wsem):
    k32, v32 = k_hbm.bitcast(u32), v_hbm.bitcast(u32)
    wq32, wo32 = wq_hbm.bitcast(u32), wo_hbm.bitcast(u32)
    wg32, wu32, wd32 = wg_hbm.bitcast(u32), wu_hbm.bitcast(u32), wd_hbm.bitcast(u32)
    cw = W // NCOL

    def start_kv(src, dst, sems, j):
        b = j // NG
        g = j % NG

        def head(i, carry):
            for c in range(NCOL):
                pltpu.make_async_copy(
                    src.at[b, g * HG + i, :, pl.ds(SK - W + c * cw, cw)],
                    dst.at[j, pl.ds(pl.multiple_of(i * DH2, 8), DH2), pl.ds(c * cw, cw)],
                    sems.at[j]).start(priority=c % 2)
            return carry

        jax.lax.fori_loop(0, HG, head, 0)

    def start_group(j):
        start_kv(k32, kbuf, ksem, j)
        start_kv(v32, vbuf, vsem, j)

    def wait_all(buf, sem):
        pltpu.make_async_copy(buf, buf, sem).wait()

    S_X, S_WR, S_WQ, S_WO, S_WG, S_WU, S_WD = range(7)

    def start_cols(src, dst, sem, ncols, piece):
        for c in range(ncols // piece):
            pltpu.make_async_copy(src.at[:, pl.ds(c * piece, piece)],
                                  dst.at[:, pl.ds(c * piece, piece)],
                                  sem).start(priority=c % 2)

    def start_rows(src, dst, sem, nrows, piece):
        for c in range(nrows // piece):
            pltpu.make_async_copy(src.at[pl.ds(c * piece, piece), :],
                                  dst.at[pl.ds(c * piece, piece), :],
                                  sem).start(priority=c % 2)

    for g in range(NG):
        start_cols(wq32.at[:, pl.ds(g * GW, GW)], wq_s.at[g], wsem.at[S_WQ], GW, 256)
    pltpu.make_async_copy(x_hbm, x_s, wsem.at[S_X]).start()
    pltpu.make_async_copy(wr_hbm, wr_s, wsem.at[S_WR]).start()
    start_rows(wo32, wo_s, wsem.at[S_WO], NG * GW2, 96)
    start_cols(wg32, wg_s, wsem.at[S_WG], F, 256)
    start_cols(wu32, wu_s, wsem.at[S_WU], F, 256)
    start_rows(wd32, wd_s, wsem.at[S_WD], F // 2, 96)

    def start_k(j):
        @pl.when(j < NJ)
        def _():
            start_kv(k32, kbuf, ksem, j)

    def start_v(j):
        @pl.when(j < NJ)
        def _():
            start_kv(v32, vbuf, vsem, j)

    start_k(0)
    start_v(0)
    start_k(1)
    start_v(1)

    wait_all(x_s, wsem.at[S_X])
    wait_all(wr_s, wsem.at[S_WR])
    x_all = x_s[...].astype(f32)
    wr = wr_s[...].astype(f32)
    wr_row = jnp.concatenate([wr[i:i + 1, :] for i in range(D // 128)], axis=1)
    wait_all(wq_s, wsem.at[S_WQ])
    wait_all(wo_s, wsem.at[S_WO])
    wait_all(wg_s, wsem.at[S_WG])
    wait_all(wu_s, wsem.at[S_WU])
    wait_all(wd_s, wsem.at[S_WD])

    row = jax.lax.broadcasted_iota(jnp.int32, (HG, GW), 0)
    col = jax.lax.broadcasted_iota(jnp.int32, (HG, GW), 1)
    mask = (col >= row * DH) & (col < row * DH + DH)
    row4 = jax.lax.broadcasted_iota(jnp.int32, (B, D), 0)

    def attention(x, b, first):
        h = _ln(x).astype(bf16)

        def group(g, acc):
            j = b * NG + g
            q = _mm(h, _as_bf16(wq_s[g]))
            qbd = jnp.where(mask, q, 0.0).astype(bf16)
            if first:
                wait_all(kbuf.at[j], ksem.at[j])

                @pl.when(g >= 1)
                def _():
                    start_k(j + 1)
            s = _mm(qbd, _as_bf16(kbuf[j])) * SCALE
            m = jnp.max(s, axis=-1, keepdims=True)
            p = jnp.exp(s - m)
            l = jnp.sum(p, axis=-1, keepdims=True)
            if first:
                wait_all(vbuf.at[j], vsem.at[j])

                @pl.when(g >= 1)
                def _():
                    start_v(j + 1)
            o = jax.lax.dot_general(p.astype(bf16), _as_bf16(vbuf[j]),
                                    (((1,), (1,)), ((), ())), preferred_element_type=f32)
            om = jnp.where(mask, o / l, 0.0).astype(bf16)
            acc = acc + _mm(om, _as_bf16(wo_s[pl.ds(pl.multiple_of(g * GW2, 8), GW2), :]))
            return acc

        acc = jax.lax.fori_loop(0, NG, group, jnp.zeros((HG, D), f32))
        return x + jnp.broadcast_to(jnp.sum(acc, axis=0, keepdims=True), (HG, D))

    lane = jax.lax.broadcasted_iota(jnp.int32, (HG, 128), 1)
    sub = jax.lax.broadcasted_iota(jnp.int32, (HG, 128), 0)
    dl = lane - 2 * sub
    NT = GW // 128

    def attention2(x, b):
        h = _ln(x).astype(bf16)
        st = {'acc': None}

        def tile_mask(t):
            c = lane + 128 * t
            return (c >= sub * DH) & (c < sub * DH + DH)

        def q_tile(u):
            g, t = divmod(u, NT)
            q = _mm(h, _as_bf16(wq_s[g, :, pl.ds(128 * t, 128)]))
            st['q', u] = jnp.where(tile_mask(t), q, 0.0).astype(bf16)

        def s_tile(u):
            g, t = divmod(u, NT)
            d = _mm(st.pop(('q', u)), _as_bf16(kbuf[b * NG + g, pl.ds(64 * t, 64), :]))
            st['s', g] = d if t == 0 else st['s', g] + d
            if t == NT - 1:
                sa = st.pop(('s', g)) * SCALE
                m = jnp.max(sa, axis=-1, keepdims=True)
                p = jnp.exp(sa - m)
                l = jnp.sum(p, axis=-1, keepdims=True)
                st['p', g] = p / l

        def v_tile(u):
            g, t = divmod(u, NT)
            p = st['p', g]
            tile = jnp.zeros((HG, 128), f32)
            for c in range(128 * t, 128 * t + 128, 16):
                hh, r = c // DH, (c % DH) // 16
                if ('pb', g, hh) not in st:
                    st['pb', g, hh] = [jnp.broadcast_to(p[hh:hh + 1, 128 * i:128 * (i + 1)], (HG, 128))
                                       for i in range(W // 128)]
                pb = st['pb', g, hh]
                acc = []
                for half in range(2):
                    alo = ahi = None
                    for i in range(4 * half, 4 * half + 4):
                        w = vbuf[b * NG + g, pl.ds(hh * DH2 + 8 * r, 8), pl.ds(128 * i, 128)]
                        lo = pltpu.bitcast(w << 16, f32) * pb[i]
                        hi = pltpu.bitcast(w & jnp.uint32(0xFFFF0000), f32) * pb[i]
                        alo = lo if alo is None else alo + lo
                        ahi = hi if ahi is None else ahi + hi
                    acc.append((alo, ahi))
                rlo = jnp.sum(acc[0][0], axis=-1, keepdims=True) + jnp.sum(acc[1][0], axis=-1, keepdims=True)
                rhi = jnp.sum(acc[0][1], axis=-1, keepdims=True) + jnp.sum(acc[1][1], axis=-1, keepdims=True)
                base = c % 128
                tile = jnp.where(dl == base, rlo, jnp.where(dl == base + 1, rhi, tile))
            st['t', u] = tile.astype(bf16)

        def w_tile(u):
            g, t = divmod(u, NT)
            d = _mm(st.pop(('t', u)), _as_bf16(wo_s[pl.ds(g * GW2 + 64 * t, 64), :]))
            st['acc'] = d if st['acc'] is None else st['acc'] + d

        N = NG * NT
        for m in range(-NT - QLEAD, N + WLAG):
            if 0 <= m + NT + QLEAD < N:
                q_tile(m + NT + QLEAD)
            if 0 <= m + NT < N:
                s_tile(m + NT)
            if 0 <= m < N:
                v_tile(m)
            if 0 <= m - WLAG < N:
                w_tile(m - WLAG)
        acc = st['acc']
        return x + jnp.broadcast_to(jnp.sum(acc, axis=0, keepdims=True), (HG, D))

    def ffn(x):
        h = _ln(x)
        r = jnp.sum(h * wr_row, axis=-1, keepdims=True)
        hb = h.astype(bf16)
        g = _mm(hb, _as_bf16(wg_s[...]))
        u = _mm(hb, _as_bf16(wu_s[...]))
        a = (g * jax.nn.sigmoid(g) * u).astype(bf16)
        y = _mm(a, _as_bf16(wd_s[...]))
        return x + h + y * jax.nn.sigmoid(r)

    def batch(b, out):
        xb = jnp.sum(jnp.where(row4 == b, x_all, 0.0), axis=0, keepdims=True)
        x = jnp.broadcast_to(xb, (HG, D))
        x = attention(x, b, True)

        x = ffn(x)
        start_k(b * NG + 5)
        x = attention2(x, b)
        start_v(b * NG + 5)
        x = ffn(x)
        return jnp.where(row4 == b, x[:B, :], out)

    out = jax.lax.fori_loop(0, B, batch, jnp.zeros((B, D), f32))
    o_ref[...] = out.astype(o_ref.dtype)


@jax.jit
def pallas_interleave_layers__sliding_block_cached__moe_arch_mod__decode_kernel(
    A_x: jax.Array,
    A_k_cache: jax.Array,
    A_v_cache: jax.Array,
    A_wq: jax.Array,
    A_wo: jax.Array,
    B_x: jax.Array,
    B_w_r: jax.Array,
    B_w_gate: jax.Array,
    B_w_up: jax.Array,
    B_w_down: jax.Array,
):
    del B_x
    k_t = jnp.transpose(A_k_cache, (0, 1, 3, 2))
    v_t = jnp.transpose(A_v_cache, (0, 1, 3, 2))
    any_spec = pl.BlockSpec(memory_space=pl.ANY)
    out = pl.pallas_call(
        _kernel,
        out_shape=jax.ShapeDtypeStruct((B, D), A_x.dtype),
        in_specs=[any_spec] * 9,
        out_specs=pl.BlockSpec(memory_space=pltpu.VMEM),
        scratch_shapes=[
            pltpu.VMEM((NJ, GW2, W), u32),
            pltpu.VMEM((NJ, GW2, W), u32),
            pltpu.VMEM((NG, D // 2, GW), u32),
            pltpu.VMEM((NG * GW2, D), u32),
            pltpu.VMEM((D // 2, F), u32),
            pltpu.VMEM((D // 2, F), u32),
            pltpu.VMEM((F // 2, D), u32),
            pltpu.VMEM((B, D), bf16),
            pltpu.VMEM((D // 128, 128), bf16),
            pltpu.SemaphoreType.DMA((NJ,)),
            pltpu.SemaphoreType.DMA((NJ,)),
            pltpu.SemaphoreType.DMA((8,)),
        ],
        compiler_params=pltpu.CompilerParams(vmem_limit_bytes=126 * 1024 * 1024),
    )(A_x.reshape(B, D), B_w_r.reshape(D // 128, 128), k_t, v_t,
      A_wq, A_wo, B_w_gate, B_w_up, B_w_down)
    return out.reshape(B, 1, D)
```

```python
import jax
import jax.numpy as jnp
from jax.experimental import pallas as pl
from jax.experimental.pallas import tpu as pltpu

B, D, H, DH, SK, F = 4, 640, 32, 192, 4096, 1536
W = min(4096, max(256, SK // 4))
HG = 8
NG = H // HG
NJ = B * NG
GW = HG * DH
DH2 = DH // 2
NC = W // 128
NT = GW // 128
ND = D // 128
NF = F // 128
EPS = 1e-5
SCALE = DH ** -0.5
QLEAD = 2
WLAG = 48

f32, bf16, u32 = jnp.float32, jnp.bfloat16, jnp.uint32


def _ln(x):
    m = jnp.mean(x, axis=-1, keepdims=True)
    xc = x - m
    v = jnp.mean(xc * xc, axis=-1, keepdims=True)
    return xc / jnp.sqrt(v + EPS)


def _as_bf16(w):
    return pltpu.bitcast(w, bf16)


def _mm(a, w):
    return jnp.dot(a, w, preferred_element_type=f32)


def _kernel(x_hbm, wr_hbm, k_hbm, v_hbm, wq_hbm, wo_hbm, wg_hbm, wu_hbm, wd_hbm,
            o_ref,
            kbuf, vbuf, wq_b, wo_b, wg_b, wu_b, wd_b, x_s, wr_s,
            ksem, vsem, wsem):
    k32, v32 = kbuf.bitcast(u32), vbuf.bitcast(u32)
    wq32, wo32 = wq_b.bitcast(u32), wo_b.bitcast(u32)
    wg32, wu32, wd32 = wg_b.bitcast(u32), wu_b.bitcast(u32), wd_b.bitcast(u32)

    def start_kv(src, dst, sems, j, hp):
        b = j // NG
        g = j % NG

        def heads(i, carry):
            for c in range(NC):
                pltpu.make_async_copy(
                    src.at[b, pl.ds(g * HG + i * hp, hp), :, pl.ds(SK - W + c * 128, 128)],
                    dst.at[j, c, pl.ds(i * hp, hp)],
                    sems.at[j]).start(priority=c % 2)
            return carry

        jax.lax.fori_loop(0, HG // hp, heads, 0)

    def start_k(j, hp=1):
        @pl.when(j < NJ)
        def _():
            start_kv(k_hbm, kbuf, ksem, j, hp)

    def start_v(j, hp=1):
        @pl.when(j < NJ)
        def _():
            start_kv(v_hbm, vbuf, vsem, j, hp)

    def wait_all(buf, sem):
        pltpu.make_async_copy(buf, buf, sem).wait()

    S_X, S_WR, S_WQ, S_WO, S_WG, S_WU, S_WD = range(7)

    def start_w(src, dst, sem, rp):
        rows, cols = src.shape
        n = 0
        for r in range(rows // rp):
            for c in range(cols // 128):
                pltpu.make_async_copy(src.at[pl.ds(r * rp, rp), pl.ds(c * 128, 128)],
                                      dst.at[c, pl.ds(r * rp, rp), :],
                                      sem).start(priority=n % 2)
                n += 1

    pltpu.make_async_copy(x_hbm, x_s, wsem.at[S_X]).start()
    pltpu.make_async_copy(wr_hbm, wr_s, wsem.at[S_WR]).start()
    start_w(wq_hbm, wq_b, wsem.at[S_WQ], 320)
    start_w(wo_hbm, wo_b, wsem.at[S_WO], 96)
    start_w(wg_hbm, wg_b, wsem.at[S_WG], 320)
    start_w(wu_hbm, wu_b, wsem.at[S_WU], 320)
    start_w(wd_hbm, wd_b, wsem.at[S_WD], 96)
    start_k(0)
    start_v(0)
    start_k(1)
    start_v(1)

    wait_all(x_s, wsem.at[S_X])
    wait_all(wr_s, wsem.at[S_WR])
    x_all = x_s[...].astype(f32)
    wr = wr_s[...].astype(f32)
    wr_row = jnp.concatenate([wr[i:i + 1, :] for i in range(ND)], axis=1)
    wait_all(wq_b, wsem.at[S_WQ])
    wait_all(wo_b, wsem.at[S_WO])
    wait_all(wg_b, wsem.at[S_WG])
    wait_all(wu_b, wsem.at[S_WU])
    wait_all(wd_b, wsem.at[S_WD])

    row = jax.lax.broadcasted_iota(jnp.int32, (HG, GW), 0)
    col = jax.lax.broadcasted_iota(jnp.int32, (HG, GW), 1)
    mask = (col >= row * DH) & (col < row * DH + DH)
    row4 = jax.lax.broadcasted_iota(jnp.int32, (B, D), 0)

    def wo_proj(t, r0, nr):
        return jnp.concatenate(
            [_mm(t, _as_bf16(wo32[n, pl.ds(r0, nr), :])) for n in range(ND)], axis=1)

    def attention1(x, b):
        h = _ln(x).astype(bf16)

        def group(g, acc):
            j = b * NG + g
            q = jnp.concatenate(
                [_mm(h, _as_bf16(wq32[g * NT + t])) for t in range(NT)], axis=1)
            qbd = jnp.where(mask, q, 0.0).astype(bf16)
            wait_all(kbuf.at[j], ksem.at[j])

            @pl.when(g == 1)
            def _():
                start_k(j + 1)

            @pl.when(g == 2)
            def _():
                start_k(j + 1)

            @pl.when(g == 3)
            def _():
                start_k(j + 1)
            s = jnp.concatenate(
                [_mm(qbd, _as_bf16(k32[j, c].reshape(HG * DH2, 128))) for c in range(NC)],
                axis=1) * SCALE
            m = jnp.max(s, axis=-1, keepdims=True)
            p = jnp.exp(s - m)
            l = jnp.sum(p, axis=-1, keepdims=True)
            wait_all(vbuf.at[j], vsem.at[j])

            @pl.when((g == 1) | (g == 2))
            def _():
                start_v(j + 1)

            @pl.when(g == 3)
            def _():
                start_v(j + 1, 2)
            pb = p.astype(bf16)
            o = None
            for c in range(NC):
                d = jax.lax.dot_general(
                    pb[:, 128 * c:128 * (c + 1)], _as_bf16(v32[j, c].reshape(HG * DH2, 128)),
                    (((1,), (1,)), ((), ())), preferred_element_type=f32)
                o = d if o is None else o + d
            om = jnp.where(mask, o / l, 0.0).astype(bf16)
            return acc + wo_proj(om, pl.multiple_of(g * (GW // 2), 8), GW // 2)

        acc = jax.lax.fori_loop(0, NG, group, jnp.zeros((HG, D), f32))
        return x + jnp.broadcast_to(jnp.sum(acc, axis=0, keepdims=True), (HG, D))

    lane = jax.lax.broadcasted_iota(jnp.int32, (HG, 128), 1)
    sub = jax.lax.broadcasted_iota(jnp.int32, (HG, 128), 0)
    dl = lane - 2 * sub

    def attention2(x, b):
        h = _ln(x).astype(bf16)
        st = {'acc': None}

        def tile_mask(t):
            c = lane + 128 * t
            return (c >= sub * DH) & (c < sub * DH + DH)

        def q_tile(u):
            g, t = divmod(u, NT)
            q = _mm(h, _as_bf16(wq32[u]))
            st['q', u] = jnp.where(tile_mask(t), q, 0.0).astype(bf16)

        def k_rows(g, c, t):
            h0, r0 = divmod(64 * t, DH2)
            j = b * NG + g
            if r0 + 64 <= DH2:
                return k32[j, c, h0, pl.ds(r0, 64), :]
            return jnp.concatenate([k32[j, c, h0, pl.ds(r0, DH2 - r0), :],
                                    k32[j, c, h0 + 1, pl.ds(0, 64 - (DH2 - r0)), :]], axis=0)

        def s_tile(u):
            g, t = divmod(u, NT)
            qt = st.pop(('q', u))
            d = jnp.concatenate([_mm(qt, _as_bf16(k_rows(g, c, t))) for c in range(NC)], axis=1)
            st['s', g] = d if t == 0 else st['s', g] + d
            if t == NT - 1:
                sa = st.pop(('s', g)) * SCALE
                m = jnp.max(sa, axis=-1, keepdims=True)
                p = jnp.exp(sa - m)
                l = jnp.sum(p, axis=-1, keepdims=True)
                st['p', g] = p / l

        def v_tile(u):
            g, t = divmod(u, NT)
            p = st['p', g]
            tile = jnp.zeros((HG, 128), f32)
            for c in range(128 * t, 128 * t + 128, 16):
                hh, r = c // DH, (c % DH) // 16
                if ('pb', g, hh) not in st:
                    st['pb', g, hh] = [jnp.broadcast_to(p[hh:hh + 1, 128 * i:128 * (i + 1)], (HG, 128))
                                       for i in range(NC)]
                pb = st['pb', g, hh]
                acc = []
                for half in range(2):
                    alo = ahi = None
                    for i in range(4 * half, 4 * half + 4):
                        w = v32[b * NG + g, i, hh, pl.ds(8 * r, 8), :]
                        lo = pltpu.bitcast(w << 16, f32) * pb[i]
                        hi = pltpu.bitcast(w & jnp.uint32(0xFFFF0000), f32) * pb[i]
                        alo = lo if alo is None else alo + lo
                        ahi = hi if ahi is None else ahi + hi
                    acc.append((alo, ahi))
                rlo = jnp.sum(acc[0][0], axis=-1, keepdims=True) + jnp.sum(acc[1][0], axis=-1, keepdims=True)
                rhi = jnp.sum(acc[0][1], axis=-1, keepdims=True) + jnp.sum(acc[1][1], axis=-1, keepdims=True)
                base = c % 128
                tile = jnp.where(dl == base, rlo, jnp.where(dl == base + 1, rhi, tile))
            st['t', u] = tile.astype(bf16)

        def w_tile(u):
            d = wo_proj(st.pop(('t', u)), 64 * u, 64)
            st['acc'] = d if st['acc'] is None else st['acc'] + d

        N = NG * NT
        for m in range(-NT - QLEAD, N + WLAG):
            if 0 <= m + NT + QLEAD < N:
                q_tile(m + NT + QLEAD)
            if 0 <= m + NT < N:
                s_tile(m + NT)
            if 0 <= m < N:
                v_tile(m)
            if 0 <= m - WLAG < N:
                w_tile(m - WLAG)
        acc = st['acc']
        return x + jnp.broadcast_to(jnp.sum(acc, axis=0, keepdims=True), (HG, D))

    def ffn(x):
        h = _ln(x)
        r = jnp.sum(h * wr_row, axis=-1, keepdims=True)
        hb = h.astype(bf16)
        g = jnp.concatenate([_mm(hb, _as_bf16(wg32[t])) for t in range(NF)], axis=1)
        u = jnp.concatenate([_mm(hb, _as_bf16(wu32[t])) for t in range(NF)], axis=1)
        a = (g * jax.nn.sigmoid(g) * u).astype(bf16)
        y = jnp.concatenate([_mm(a, _as_bf16(wd32[n])) for n in range(ND)], axis=1)
        return x + h + y * jax.nn.sigmoid(r)

    def batch(b, out):
        xb = jnp.sum(jnp.where(row4 == b, x_all, 0.0), axis=0, keepdims=True)
        x = jnp.broadcast_to(xb, (HG, D))
        x = attention1(x, b)
        x = ffn(x)
        start_k(b * NG + 5, 2)
        x = attention2(x, b)
        start_v(b * NG + 5, 2)
        x = ffn(x)
        return jnp.where(row4 == b, x[:B, :], out)

    out = jax.lax.fori_loop(0, B, batch, jnp.zeros((B, D), f32))
    o_ref[...] = out.astype(o_ref.dtype)


@jax.jit
def pallas_interleave_layers__sliding_block_cached__moe_arch_mod__decode_kernel(
    A_x: jax.Array,
    A_k_cache: jax.Array,
    A_v_cache: jax.Array,
    A_wq: jax.Array,
    A_wo: jax.Array,
    B_x: jax.Array,
    B_w_r: jax.Array,
    B_w_gate: jax.Array,
    B_w_up: jax.Array,
    B_w_down: jax.Array,
):
    del B_x
    k_t = jnp.transpose(A_k_cache, (0, 1, 3, 2))
    v_t = jnp.transpose(A_v_cache, (0, 1, 3, 2))
    any_spec = pl.BlockSpec(memory_space=pl.ANY)
    out = pl.pallas_call(
        _kernel,
        out_shape=jax.ShapeDtypeStruct((B, D), A_x.dtype),
        in_specs=[any_spec] * 9,
        out_specs=pl.BlockSpec(memory_space=pltpu.VMEM),
        scratch_shapes=[
            pltpu.VMEM((NJ, NC, HG, DH, 128), bf16),
            pltpu.VMEM((NJ, NC, HG, DH, 128), bf16),
            pltpu.VMEM((H * DH // 128, D, 128), bf16),
            pltpu.VMEM((ND, H * DH, 128), bf16),
            pltpu.VMEM((NF, D, 128), bf16),
            pltpu.VMEM((NF, D, 128), bf16),
            pltpu.VMEM((ND, F, 128), bf16),
            pltpu.VMEM((B, D), bf16),
            pltpu.VMEM((ND, 128), bf16),
            pltpu.SemaphoreType.DMA((NJ,)),
            pltpu.SemaphoreType.DMA((NJ,)),
            pltpu.SemaphoreType.DMA((8,)),
        ],
        compiler_params=pltpu.CompilerParams(vmem_limit_bytes=126 * 1024 * 1024),
    )(A_x.reshape(B, D), B_w_r.reshape(ND, 128), k_t, v_t,
      A_wq, A_wo, B_w_gate, B_w_up, B_w_down)
    return out.reshape(B, 1, D)
```

```python
import jax
import jax.numpy as jnp
from jax.experimental import pallas as pl
from jax.experimental.pallas import tpu as pltpu

B, D, H, DH, SK, F = 4, 640, 32, 192, 4096, 1536
W = min(4096, max(256, SK // 4))
HG = 8
NG = H // HG
NJ = B * NG
GW = HG * DH
DH2 = DH // 2
NC = W // 128
NT = GW // 128
ND = D // 128
NF = F // 128
EPS = 1e-5
SCALE = DH ** -0.5
VP = 2
QLEAD = 2
WLAG = 48

f32, bf16, u32 = jnp.float32, jnp.bfloat16, jnp.uint32


def _ln(x):
    m = jnp.mean(x, axis=-1, keepdims=True)
    xc = x - m
    v = jnp.mean(xc * xc, axis=-1, keepdims=True)
    return xc / jnp.sqrt(v + EPS)


def _as_bf16(w):
    return pltpu.bitcast(w, bf16)


def _mm(a, w):
    return jnp.dot(a, w, preferred_element_type=f32)


def _kernel(x_hbm, wr_hbm, k_hbm, v_hbm, wq_hbm, wo_hbm, wg_hbm, wu_hbm, wd_hbm,
            o_ref,
            kbuf, vbuf, wq_b, wo_b, wg_b, wu_b, wd_b, x_s, wr_s,
            ksem, vsem, wsem):
    k32, v32 = kbuf.bitcast(u32), vbuf.bitcast(u32)
    wq32, wo32 = wq_b.bitcast(u32), wo_b.bitcast(u32)
    wg32, wu32, wd32 = wg_b.bitcast(u32), wu_b.bitcast(u32), wd_b.bitcast(u32)

    def start_kv(src, dst, sems, j, hp, sem_heads):
        b = j // NG
        g = j % NG

        def heads(i, carry):
            sem = sems.at[j * (HG // sem_heads) + (i * hp) // sem_heads]
            for c in range(NC):
                pltpu.make_async_copy(
                    src.at[b, pl.ds(g * HG + i * hp, hp), :, pl.ds(SK - W + c * 128, 128)],
                    dst.at[j, c, pl.ds(i * hp, hp)],
                    sem).start(priority=c % 2)
            return carry

        jax.lax.fori_loop(0, HG // hp, heads, 0)

    def start_k(j, hp=1):
        if isinstance(j, int):
            if j < NJ:
                start_kv(k_hbm, kbuf, ksem, j, hp, HG)
            return

        @pl.when(j < NJ)
        def _():
            start_kv(k_hbm, kbuf, ksem, j, hp, HG)

    def start_v(j, hp=1):
        if isinstance(j, int):
            if j < NJ:
                start_kv(v_hbm, vbuf, vsem, j, hp, VP)
            return

        @pl.when(j < NJ)
        def _():
            start_kv(v_hbm, vbuf, vsem, j, hp, VP)

    def wait_all(buf, sem):
        pltpu.make_async_copy(buf, buf, sem).wait()

    S_X, S_WR, S_WQ, S_WO, S_WG, S_WU, S_WD = range(7)

    def start_w(src, dst, sem, rp):
        rows, cols = src.shape
        n = 0
        for r in range(rows // rp):
            for c in range(cols // 128):
                pltpu.make_async_copy(src.at[pl.ds(r * rp, rp), pl.ds(c * 128, 128)],
                                      dst.at[c, pl.ds(r * rp, rp), :],
                                      sem).start(priority=n % 2)
                n += 1

    pltpu.make_async_copy(x_hbm, x_s, wsem.at[S_X]).start()
    pltpu.make_async_copy(wr_hbm, wr_s, wsem.at[S_WR]).start()
    start_w(wq_hbm, wq_b, wsem.at[S_WQ], 320)
    start_w(wo_hbm, wo_b, wsem.at[S_WO], 96)
    start_w(wg_hbm, wg_b, wsem.at[S_WG], 320)
    start_w(wu_hbm, wu_b, wsem.at[S_WU], 320)
    start_w(wd_hbm, wd_b, wsem.at[S_WD], 96)
    start_k(0)
    start_v(0)
    start_k(1)
    start_v(1)

    wait_all(x_s, wsem.at[S_X])
    wait_all(wr_s, wsem.at[S_WR])
    x_all = x_s[...].astype(f32)
    wr = wr_s[...].astype(f32)
    wr_row = jnp.concatenate([wr[i:i + 1, :] for i in range(ND)], axis=1)
    wait_all(wq_b, wsem.at[S_WQ])
    wait_all(wo_b, wsem.at[S_WO])
    wait_all(wg_b, wsem.at[S_WG])
    wait_all(wu_b, wsem.at[S_WU])
    wait_all(wd_b, wsem.at[S_WD])

    row = jax.lax.broadcasted_iota(jnp.int32, (HG, GW), 0)
    col = jax.lax.broadcasted_iota(jnp.int32, (HG, GW), 1)
    mask = (col >= row * DH) & (col < row * DH + DH)
    row4 = jax.lax.broadcasted_iota(jnp.int32, (B, D), 0)

    def wo_proj(t, r0, nr):
        return jnp.concatenate(
            [_mm(t, _as_bf16(wo32[n, pl.ds(r0, nr), :])) for n in range(ND)], axis=1)

    def attention1(x, b):
        h = _ln(x).astype(bf16)

        def group(g, acc):
            j = b * NG + g
            q = jnp.concatenate(
                [_mm(h, _as_bf16(wq32[g * NT + t])) for t in range(NT)], axis=1)
            qbd = jnp.where(mask, q, 0.0).astype(bf16)
            wait_all(kbuf.at[j], ksem.at[j])

            @pl.when(g == 1)
            def _():
                start_k(j + 1)

            @pl.when(g == 2)
            def _():
                start_k(j + 1)

            @pl.when(g == 3)
            def _():
                start_k(j + 1)
            s = jnp.concatenate(
                [_mm(qbd, _as_bf16(k32[j, c].reshape(HG * DH2, 128))) for c in range(NC)],
                axis=1) * SCALE
            m = jnp.max(s, axis=-1, keepdims=True)
            p = jnp.exp(s - m)
            l = jnp.sum(p, axis=-1, keepdims=True)
            pb = p.astype(bf16)
            rl = 1.0 / l
            for part in range(HG // VP):
                wait_all(vbuf.at[j, :, pl.ds(part * VP, VP)], vsem.at[j * (HG // VP) + part])
                if part == HG // VP - 1:
                    @pl.when((g == 1) | (g == 2))
                    def _():
                        start_v(j + 1)

                    @pl.when(g == 3)
                    def _():
                        start_v(j + 1, 2)
                o = None
                for c in range(NC):
                    d = jax.lax.dot_general(
                        pb[:, 128 * c:128 * (c + 1)],
                        _as_bf16(v32[j, c, pl.ds(part * VP, VP)].reshape(VP * DH2, 128)),
                        (((1,), (1,)), ((), ())), preferred_element_type=f32)
                    o = d if o is None else o + d
                cols = slice(part * VP * DH, (part + 1) * VP * DH)
                om = jnp.where(mask[:, cols], o * rl, 0.0).astype(bf16)
                acc = acc + wo_proj(om, pl.multiple_of(g * (GW // 2) + part * VP * DH2, 8), VP * DH2)
            return acc

        acc = jax.lax.fori_loop(0, NG, group, jnp.zeros((HG, D), f32))
        return x + jnp.broadcast_to(jnp.sum(acc, axis=0, keepdims=True), (HG, D))

    lane = jax.lax.broadcasted_iota(jnp.int32, (HG, 128), 1)
    sub = jax.lax.broadcasted_iota(jnp.int32, (HG, 128), 0)
    dl = lane - 2 * sub

    def attention2(x, b):
        h = _ln(x).astype(bf16)
        st = {'acc': None}

        def tile_mask(t):
            c = lane + 128 * t
            return (c >= sub * DH) & (c < sub * DH + DH)

        def q_tile(u):
            g, t = divmod(u, NT)
            q = _mm(h, _as_bf16(wq32[u]))
            st['q', u] = jnp.where(tile_mask(t), q, 0.0).astype(bf16)

        def k_rows(g, c, t):
            h0, r0 = divmod(64 * t, DH2)
            j = b * NG + g
            if r0 + 64 <= DH2:
                return k32[j, c, h0, pl.ds(r0, 64), :]
            return jnp.concatenate([k32[j, c, h0, pl.ds(r0, DH2 - r0), :],
                                    k32[j, c, h0 + 1, pl.ds(0, 64 - (DH2 - r0)), :]], axis=0)

        def s_tile(u):
            g, t = divmod(u, NT)
            qt = st.pop(('q', u))
            d = jnp.concatenate([_mm(qt, _as_bf16(k_rows(g, c, t))) for c in range(NC)], axis=1)
            st['s', g] = d if t == 0 else st['s', g] + d
            if t == NT - 1:
                sa = st.pop(('s', g)) * SCALE
                m = jnp.max(sa, axis=-1, keepdims=True)
                p = jnp.exp(sa - m)
                l = jnp.sum(p, axis=-1, keepdims=True)
                st['p', g] = p / l

        def v_tile(u):
            g, t = divmod(u, NT)
            p = st['p', g]
            tile = jnp.zeros((HG, 128), f32)
            for c in range(128 * t, 128 * t + 128, 16):
                hh, r = c // DH, (c % DH) // 16
                if ('pb', g, hh) not in st:
                    st['pb', g, hh] = [jnp.broadcast_to(p[hh:hh + 1, 128 * i:128 * (i + 1)], (HG, 128))
                                       for i in range(NC)]
                pb = st['pb', g, hh]
                acc = []
                for half in range(2):
                    alo = ahi = None
                    for i in range(4 * half, 4 * half + 4):
                        w = v32[b * NG + g, i, hh, pl.ds(8 * r, 8), :]
                        lo = pltpu.bitcast(w << 16, f32) * pb[i]
                        hi = pltpu.bitcast(w & jnp.uint32(0xFFFF0000), f32) * pb[i]
                        alo = lo if alo is None else alo + lo
                        ahi = hi if ahi is None else ahi + hi
                    acc.append((alo, ahi))
                rlo = jnp.sum(acc[0][0], axis=-1, keepdims=True) + jnp.sum(acc[1][0], axis=-1, keepdims=True)
                rhi = jnp.sum(acc[0][1], axis=-1, keepdims=True) + jnp.sum(acc[1][1], axis=-1, keepdims=True)
                base = c % 128
                tile = jnp.where(dl == base, rlo, jnp.where(dl == base + 1, rhi, tile))
            st['t', u] = tile.astype(bf16)

        def w_tile(u):
            d = wo_proj(st.pop(('t', u)), 64 * u, 64)
            st['acc'] = d if st['acc'] is None else st['acc'] + d

        N = NG * NT
        for m in range(-NT - QLEAD, N + WLAG):
            if 0 <= m + NT + QLEAD < N:
                q_tile(m + NT + QLEAD)
            if 0 <= m + NT < N:
                s_tile(m + NT)
            if 0 <= m < N:
                v_tile(m)
            if 0 <= m - WLAG < N:
                w_tile(m - WLAG)
        acc = st['acc']
        return x + jnp.broadcast_to(jnp.sum(acc, axis=0, keepdims=True), (HG, D))

    def ffn(x):
        h = _ln(x)
        r = jnp.sum(h * wr_row, axis=-1, keepdims=True)
        hb = h.astype(bf16)
        g = jnp.concatenate([_mm(hb, _as_bf16(wg32[t])) for t in range(NF)], axis=1)
        u = jnp.concatenate([_mm(hb, _as_bf16(wu32[t])) for t in range(NF)], axis=1)
        a = (g * jax.nn.sigmoid(g) * u).astype(bf16)
        y = jnp.concatenate([_mm(a, _as_bf16(wd32[n])) for n in range(ND)], axis=1)
        return x + h + y * jax.nn.sigmoid(r)

    def batch(b, out):
        xb = jnp.sum(jnp.where(row4 == b, x_all, 0.0), axis=0, keepdims=True)
        x = jnp.broadcast_to(xb, (HG, D))
        x = attention1(x, b)
        x = ffn(x)
        start_k(b * NG + 5, 2)
        x = attention2(x, b)
        start_v(b * NG + 5, 2)
        x = ffn(x)
        return jnp.where(row4 == b, x[:B, :], out)

    out = jax.lax.fori_loop(0, B - 1, batch, jnp.zeros((B, D), f32))
    out = batch(B - 1, out)
    o_ref[...] = out.astype(o_ref.dtype)


@jax.jit
def pallas_interleave_layers__sliding_block_cached__moe_arch_mod__decode_kernel(
    A_x: jax.Array,
    A_k_cache: jax.Array,
    A_v_cache: jax.Array,
    A_wq: jax.Array,
    A_wo: jax.Array,
    B_x: jax.Array,
    B_w_r: jax.Array,
    B_w_gate: jax.Array,
    B_w_up: jax.Array,
    B_w_down: jax.Array,
):
    del B_x
    k_t = jnp.transpose(A_k_cache, (0, 1, 3, 2))
    v_t = jnp.transpose(A_v_cache, (0, 1, 3, 2))
    any_spec = pl.BlockSpec(memory_space=pl.ANY)
    out = pl.pallas_call(
        _kernel,
        out_shape=jax.ShapeDtypeStruct((B, D), A_x.dtype),
        in_specs=[any_spec] * 9,
        out_specs=pl.BlockSpec(memory_space=pltpu.VMEM),
        scratch_shapes=[
            pltpu.VMEM((NJ, NC, HG, DH, 128), bf16),
            pltpu.VMEM((NJ, NC, HG, DH, 128), bf16),
            pltpu.VMEM((H * DH // 128, D, 128), bf16),
            pltpu.VMEM((ND, H * DH, 128), bf16),
            pltpu.VMEM((NF, D, 128), bf16),
            pltpu.VMEM((NF, D, 128), bf16),
            pltpu.VMEM((ND, F, 128), bf16),
            pltpu.VMEM((B, D), bf16),
            pltpu.VMEM((ND, 128), bf16),
            pltpu.SemaphoreType.DMA((NJ,)),
            pltpu.SemaphoreType.DMA((NJ * HG // VP,)),
            pltpu.SemaphoreType.DMA((8,)),
        ],
        compiler_params=pltpu.CompilerParams(vmem_limit_bytes=126 * 1024 * 1024),
    )(A_x.reshape(B, D), B_w_r.reshape(ND, 128), k_t, v_t,
      A_wq, A_wo, B_w_gate, B_w_up, B_w_down)
    return out.reshape(B, 1, D)
```

```python
import jax
import jax.numpy as jnp
from jax.experimental import pallas as pl
from jax.experimental.pallas import tpu as pltpu

B, D, H, DH, SK, F = 4, 640, 32, 192, 4096, 1536
W = min(4096, max(256, SK // 4))
HG = 8
NG = H // HG
NJ = B * NG
GW = HG * DH
DH2 = DH // 2
NC = W // 128
NT = GW // 128
ND = D // 128
NF = F // 128
EPS = 1e-5
SCALE = DH ** -0.5
VP = 2
U = 2
UT = U * DH // 128
SLEAD = 4
QLEAD = 2
WLAG = 12

f32, bf16, u32 = jnp.float32, jnp.bfloat16, jnp.uint32


def _ln(x):
    m = jnp.mean(x, axis=-1, keepdims=True)
    xc = x - m
    v = jnp.mean(xc * xc, axis=-1, keepdims=True)
    return xc / jnp.sqrt(v + EPS)


def _as_bf16(w):
    return pltpu.bitcast(w, bf16)


def _mm(a, w):
    return jnp.dot(a, w, preferred_element_type=f32)


def _kernel(x_hbm, wr_hbm, k_hbm, v_hbm, wq_hbm, wo_hbm, wg_hbm, wu_hbm, wd_hbm,
            o_ref,
            kbuf, vbuf, wq_b, wo_b, wg_b, wu_b, wd_b, x_s, wr_s,
            ksem, vsem, wsem):
    k32, v32 = kbuf.bitcast(u32), vbuf.bitcast(u32)
    wq32, wo32 = wq_b.bitcast(u32), wo_b.bitcast(u32)
    wg32, wu32, wd32 = wg_b.bitcast(u32), wu_b.bitcast(u32), wd_b.bitcast(u32)

    def start_kv(src, dst, sems, j, hp, sem_heads):
        b = j // NG
        g = j % NG

        def heads(i, carry):
            sem = sems.at[(j % 2) * (HG // sem_heads) + (i * hp) // sem_heads]
            for c in range(NC):
                pltpu.make_async_copy(
                    src.at[b, pl.ds(g * HG + i * hp, hp), :, pl.ds(SK - W + c * 128, 128)],
                    dst.at[j, c, pl.ds(i * hp, hp)],
                    sem).start(priority=c % 2)
            return carry

        jax.lax.fori_loop(0, HG // hp, heads, 0)

    def start_k(j, hp=1):
        if isinstance(j, int):
            if j < NJ:
                start_kv(k_hbm, kbuf, ksem, j, hp, HG)
            return

        @pl.when(j < NJ)
        def _():
            start_kv(k_hbm, kbuf, ksem, j, hp, HG)

    def start_v(j, hp=1):
        if isinstance(j, int):
            if j < NJ:
                start_kv(v_hbm, vbuf, vsem, j, hp, VP)
            return

        @pl.when(j < NJ)
        def _():
            start_kv(v_hbm, vbuf, vsem, j, hp, VP)

    def wait_all(buf, sem):
        pltpu.make_async_copy(buf, buf, sem).wait()

    def start_w(src, dst, sem, rp):
        rows, cols = src.shape
        n = 0
        for r in range(rows // rp):
            for c in range(cols // 128):
                pltpu.make_async_copy(src.at[pl.ds(r * rp, rp), pl.ds(c * 128, 128)],
                                      dst.at[c, pl.ds(r * rp, rp), :],
                                      sem).start(priority=n % 2)
                n += 1

    pltpu.make_async_copy(x_hbm, x_s, wsem).start()
    pltpu.make_async_copy(wr_hbm, wr_s, wsem).start()
    start_w(wq_hbm, wq_b, wsem, 320)
    start_w(wo_hbm, wo_b, wsem, 96)
    start_w(wg_hbm, wg_b, wsem, 320)
    start_w(wu_hbm, wu_b, wsem, 320)
    start_w(wd_hbm, wd_b, wsem, 96)
    start_k(0)
    start_v(0)
    start_k(1)
    start_v(1)

    for buf in (x_s, wr_s, wq_b, wo_b, wg_b, wu_b, wd_b):
        wait_all(buf, wsem)
    x_all = x_s[...].astype(f32)
    wr = wr_s[...].astype(f32)
    wr_row = jnp.concatenate([wr[i:i + 1, :] for i in range(ND)], axis=1)

    row = jax.lax.broadcasted_iota(jnp.int32, (HG, GW), 0)
    col = jax.lax.broadcasted_iota(jnp.int32, (HG, GW), 1)
    mask = (col >= row * DH) & (col < row * DH + DH)
    row4 = jax.lax.broadcasted_iota(jnp.int32, (B, D), 0)

    def wo_proj(t, r0, nr):
        return jnp.concatenate(
            [_mm(t, _as_bf16(wo32[n, pl.ds(r0, nr), :])) for n in range(ND)], axis=1)

    def attention1(x, b):
        h = _ln(x).astype(bf16)

        def group(g, acc):
            j = b * NG + g
            q = jnp.concatenate(
                [_mm(h, _as_bf16(wq32[g * NT + t])) for t in range(NT)], axis=1)
            qbd = jnp.where(mask, q, 0.0).astype(bf16)
            wait_all(kbuf.at[j], ksem.at[g % 2])

            @pl.when(g == 1)
            def _():
                start_k(j + 1)

            @pl.when(g == 2)
            def _():
                start_k(j + 1)

            @pl.when(g == 3)
            def _():
                start_k(j + 1)
            s = jnp.concatenate(
                [_mm(qbd, _as_bf16(k32[j, c].reshape(HG * DH2, 128))) for c in range(NC)],
                axis=1) * SCALE
            m = jnp.max(s, axis=-1, keepdims=True)
            p = jnp.exp(s - m)
            l = jnp.sum(p, axis=-1, keepdims=True)
            pb = p.astype(bf16)
            rl = 1.0 / l
            for part in range(HG // VP):
                wait_all(vbuf.at[j, :, pl.ds(part * VP, VP)], vsem.at[(g % 2) * (HG // VP) + part])
                if part == HG // VP - 1:
                    @pl.when((g == 1) | (g == 2))
                    def _():
                        start_v(j + 1)

                    @pl.when(g == 3)
                    def _():
                        start_v(j + 1, 2)
                o = None
                for c in range(NC):
                    d = jax.lax.dot_general(
                        pb[:, 128 * c:128 * (c + 1)],
                        _as_bf16(v32[j, c, pl.ds(part * VP, VP)].reshape(VP * DH2, 128)),
                        (((1,), (1,)), ((), ())), preferred_element_type=f32)
                    o = d if o is None else o + d
                cols = slice(part * VP * DH, (part + 1) * VP * DH)
                om = jnp.where(mask[:, cols], o * rl, 0.0).astype(bf16)
                acc = acc + wo_proj(om, pl.multiple_of(g * (GW // 2) + part * VP * DH2, 8), VP * DH2)
            return acc

        acc = jax.lax.fori_loop(0, NG, group, jnp.zeros((HG, D), f32))
        return x + jnp.broadcast_to(jnp.sum(acc, axis=0, keepdims=True), (HG, D))

    lane = jax.lax.broadcasted_iota(jnp.int32, (HG, 128), 1)
    sub = jax.lax.broadcasted_iota(jnp.int32, (HG, 128), 0)
    dl = lane - 2 * sub

    def attention2(x, b):
        h = _ln(x).astype(bf16)
        st = {'acc': None}

        def tile_mask(t):
            c = lane + 128 * t
            return (c >= sub * DH) & (c < sub * DH + DH)

        def q_tile(u):
            q = _mm(h, _as_bf16(wq32[u]))
            st['q', u] = jnp.where(tile_mask(u % UT), q, 0.0).astype(bf16)

        def k_rows(c, u):
            hd, r0 = divmod(64 * u, DH2)
            g, h0 = divmod(hd, HG)
            j = b * NG + g
            if r0 + 64 <= DH2:
                return k32[j, c, h0, pl.ds(r0, 64), :]
            return jnp.concatenate([k32[j, c, h0, pl.ds(r0, DH2 - r0), :],
                                    k32[j, c, h0 + 1, pl.ds(0, 64 - (DH2 - r0)), :]], axis=0)

        def s_tile(u):
            k, t = divmod(u, UT)
            qt = st.pop(('q', u))
            d = jnp.concatenate([_mm(qt, _as_bf16(k_rows(c, u))) for c in range(NC)], axis=1)
            st['s', k] = d if t == 0 else st['s', k] + d
            if t == UT - 1:
                sa = st.pop(('s', k)) * SCALE
                m = jnp.max(sa, axis=-1, keepdims=True)
                p = jnp.exp(sa - m)
                l = jnp.sum(p, axis=-1, keepdims=True)
                st['p', k] = p / l

        def v_tile(u):
            p = st['p', u // UT]
            tile = jnp.zeros((HG, 128), f32)
            for c in range(128 * u, 128 * u + 128, 16):
                hd, r = c // DH, (c % DH) // 16
                g, hh = divmod(hd, HG)
                if ('pb', hd) not in st:
                    hu = hd % U
                    st['pb', hd] = [jnp.broadcast_to(p[hu:hu + 1, 128 * i:128 * (i + 1)], (HG, 128))
                                    for i in range(NC)]
                pb = st['pb', hd]
                acc = []
                for half in range(2):
                    alo = ahi = None
                    for i in range(4 * half, 4 * half + 4):
                        w = v32[b * NG + g, i, hh, pl.ds(8 * r, 8), :]
                        lo = pltpu.bitcast(w << 16, f32) * pb[i]
                        hi = pltpu.bitcast(w & jnp.uint32(0xFFFF0000), f32) * pb[i]
                        alo = lo if alo is None else alo + lo
                        ahi = hi if ahi is None else ahi + hi
                    acc.append((alo, ahi))
                rlo = jnp.sum(acc[0][0], axis=-1, keepdims=True) + jnp.sum(acc[1][0], axis=-1, keepdims=True)
                rhi = jnp.sum(acc[0][1], axis=-1, keepdims=True) + jnp.sum(acc[1][1], axis=-1, keepdims=True)
                base = c % 128
                tile = jnp.where(dl == base, rlo, jnp.where(dl == base + 1, rhi, tile))
            st['t', u] = tile.astype(bf16)

        def w_tile(u):
            d = wo_proj(st.pop(('t', u)), 64 * u, 64)
            st['acc'] = d if st['acc'] is None else st['acc'] + d

        N = NG * NT
        SL = SLEAD * UT
        for m in range(-SL - QLEAD, N + WLAG):
            if 0 <= m + SL + QLEAD < N:
                q_tile(m + SL + QLEAD)
            if 0 <= m + SL < N:
                s_tile(m + SL)
            if 0 <= m < N:
                v_tile(m)
            if 0 <= m - WLAG < N:
                w_tile(m - WLAG)
        acc = st['acc']
        return x + jnp.broadcast_to(jnp.sum(acc, axis=0, keepdims=True), (HG, D))

    def ffn(x):
        h = _ln(x)
        r = jnp.sum(h * wr_row, axis=-1, keepdims=True)
        hb = h.astype(bf16)
        g = jnp.concatenate([_mm(hb, _as_bf16(wg32[t])) for t in range(NF)], axis=1)
        u = jnp.concatenate([_mm(hb, _as_bf16(wu32[t])) for t in range(NF)], axis=1)
        a = (g * jax.nn.sigmoid(g) * u).astype(bf16)
        y = jnp.concatenate([_mm(a, _as_bf16(wd32[n])) for n in range(ND)], axis=1)
        return x + h + y * jax.nn.sigmoid(r)

    def batch(b, out):
        xb = jnp.sum(jnp.where(row4 == b, x_all, 0.0), axis=0, keepdims=True)
        x = jnp.broadcast_to(xb, (HG, D))
        x = attention1(x, b)
        x = ffn(x)
        start_k(b * NG + 5, 2)
        x = attention2(x, b)
        start_v(b * NG + 5, 2)
        x = ffn(x)
        return jnp.where(row4 == b, x[:B, :], out)

    out = jax.lax.fori_loop(0, B - 1, batch, jnp.zeros((B, D), f32))
    out = batch(B - 1, out)
    o_ref[...] = out.astype(o_ref.dtype)


@jax.jit
def pallas_interleave_layers__sliding_block_cached__moe_arch_mod__decode_kernel(
    A_x: jax.Array,
    A_k_cache: jax.Array,
    A_v_cache: jax.Array,
    A_wq: jax.Array,
    A_wo: jax.Array,
    B_x: jax.Array,
    B_w_r: jax.Array,
    B_w_gate: jax.Array,
    B_w_up: jax.Array,
    B_w_down: jax.Array,
):
    del B_x
    k_t = jnp.transpose(A_k_cache, (0, 1, 3, 2))
    v_t = jnp.transpose(A_v_cache, (0, 1, 3, 2))
    any_spec = pl.BlockSpec(memory_space=pl.ANY)
    out = pl.pallas_call(
        _kernel,
        out_shape=jax.ShapeDtypeStruct((B, D), A_x.dtype),
        in_specs=[any_spec] * 9,
        out_specs=pl.BlockSpec(memory_space=pltpu.VMEM),
        scratch_shapes=[
            pltpu.VMEM((NJ, NC, HG, DH, 128), bf16),
            pltpu.VMEM((NJ, NC, HG, DH, 128), bf16),
            pltpu.VMEM((H * DH // 128, D, 128), bf16),
            pltpu.VMEM((ND, H * DH, 128), bf16),
            pltpu.VMEM((NF, D, 128), bf16),
            pltpu.VMEM((NF, D, 128), bf16),
            pltpu.VMEM((ND, F, 128), bf16),
            pltpu.VMEM((B, D), bf16),
            pltpu.VMEM((ND, 128), bf16),
            pltpu.SemaphoreType.DMA((2,)),
            pltpu.SemaphoreType.DMA((2 * HG // VP,)),
            pltpu.SemaphoreType.DMA(()),
        ],
        compiler_params=pltpu.CompilerParams(vmem_limit_bytes=126 * 1024 * 1024),
    )(A_x.reshape(B, D), B_w_r.reshape(ND, 128), k_t, v_t,
      A_wq, A_wo, B_w_gate, B_w_up, B_w_down)
    return out.reshape(B, 1, D)
```

```python
import jax
import jax.numpy as jnp
from jax.experimental import pallas as pl
from jax.experimental.pallas import tpu as pltpu

B, D, H, DH, SK, F = 4, 640, 32, 192, 4096, 1536
W = min(4096, max(256, SK // 4))
HG = 8
NG = H // HG
NJ = B * NG
GW = HG * DH
DH2 = DH // 2
NC = W // 128
NT = GW // 128
ND = D // 128
NF = F // 128
EPS = 1e-5
SCALE = DH ** -0.5
LOG2E = 1.4426950408889634
VP = 2
U = 4
UT = U * DH // 128
SLEAD = 2
QLEAD = 2
WLAG = 24

f32, bf16, u32 = jnp.float32, jnp.bfloat16, jnp.uint32


def _ln(x):
    m = jnp.mean(x, axis=-1, keepdims=True)
    m2 = jnp.mean(x * x, axis=-1, keepdims=True)
    v = jnp.maximum(m2 - m * m, 0.0)
    return (x - m) * jax.lax.rsqrt(v + EPS)


def _as_bf16(w):
    return pltpu.bitcast(w, bf16)


def _mm(a, w):
    return jnp.dot(a, w, preferred_element_type=f32)


def _kernel(x_hbm, wr_hbm, k_hbm, v_hbm, wq_hbm, wo_hbm, wg_hbm, wu_hbm, wd_hbm,
            o_ref,
            kbuf, vbuf, wq_b, wo_b, wg_b, wu_b, wd_b, x_s, wr_s,
            ksem, vsem, wsem):
    k32, v32 = kbuf.bitcast(u32), vbuf.bitcast(u32)
    wq32, wo32 = wq_b.bitcast(u32), wo_b.bitcast(u32)
    wg32, wu32, wd32 = wg_b.bitcast(u32), wu_b.bitcast(u32), wd_b.bitcast(u32)

    def start_kv(src, dst, sems, j, hp, sem_heads):
        b = j // NG
        g = j % NG

        def heads(i, carry):
            sem = sems.at[(j % 2) * (HG // sem_heads) + (i * hp) // sem_heads]
            for c in range(NC):
                pltpu.make_async_copy(
                    src.at[b, pl.ds(g * HG + i * hp, hp), :, pl.ds(SK - W + c * 128, 128)],
                    dst.at[j, c, pl.ds(i * hp, hp)],
                    sem).start(priority=c % 2)
            return carry

        jax.lax.fori_loop(0, HG // hp, heads, 0)

    def start_k(j, hp=1):
        if isinstance(j, int):
            if j < NJ:
                start_kv(k_hbm, kbuf, ksem, j, hp, HG)
            return

        @pl.when(j < NJ)
        def _():
            start_kv(k_hbm, kbuf, ksem, j, hp, HG)

    def start_v(j, hp=1):
        if isinstance(j, int):
            if j < NJ:
                start_kv(v_hbm, vbuf, vsem, j, hp, VP)
            return

        @pl.when(j < NJ)
        def _():
            start_kv(v_hbm, vbuf, vsem, j, hp, VP)

    def wait_all(buf, sem):
        pltpu.make_async_copy(buf, buf, sem).wait()

    def start_w(src, dst, sem, rp):
        rows, cols = src.shape
        n = 0
        for r in range(rows // rp):
            for c in range(cols // 128):
                pltpu.make_async_copy(src.at[pl.ds(r * rp, rp), pl.ds(c * 128, 128)],
                                      dst.at[c, pl.ds(r * rp, rp), :],
                                      sem).start(priority=n % 2)
                n += 1

    pltpu.make_async_copy(x_hbm, x_s, wsem).start()
    pltpu.make_async_copy(wr_hbm, wr_s, wsem).start()
    start_w(wq_hbm, wq_b, wsem, 320)
    start_w(wo_hbm, wo_b, wsem, 96)
    start_w(wg_hbm, wg_b, wsem, 320)
    start_w(wu_hbm, wu_b, wsem, 320)
    start_w(wd_hbm, wd_b, wsem, 96)
    start_k(0)
    start_v(0)
    start_k(1)
    start_v(1)

    for buf in (x_s, wr_s, wq_b, wo_b, wg_b, wu_b, wd_b):
        wait_all(buf, wsem)
    x_all = x_s[...].astype(f32)
    wr = wr_s[...].astype(f32)
    wr_row = jnp.concatenate([wr[i:i + 1, :] for i in range(ND)], axis=1)

    row = jax.lax.broadcasted_iota(jnp.int32, (HG, GW), 0)
    col = jax.lax.broadcasted_iota(jnp.int32, (HG, GW), 1)
    mask = (col >= row * DH) & (col < row * DH + DH)
    row4 = jax.lax.broadcasted_iota(jnp.int32, (B, D), 0)

    def wo_proj(t, r0, nr):
        return jnp.concatenate(
            [_mm(t, _as_bf16(wo32[n, pl.ds(r0, nr), :])) for n in range(ND)], axis=1)

    def attention1(x, b):
        h = _ln(x).astype(bf16)

        def group(g, acc):
            j = b * NG + g
            q = jnp.concatenate(
                [_mm(h, _as_bf16(wq32[g * NT + t])) for t in range(NT)], axis=1)
            qbd = jnp.where(mask, q, 0.0).astype(bf16)
            wait_all(kbuf.at[j], ksem.at[g % 2])

            @pl.when(g == 1)
            def _():
                start_k(j + 1)

            @pl.when(g == 2)
            def _():
                start_k(j + 1)

            @pl.when(g == 3)
            def _():
                start_k(j + 1)
            s = jnp.concatenate(
                [_mm(qbd, _as_bf16(k32[j, c].reshape(HG * DH2, 128))) for c in range(NC)],
                axis=1) * SCALE
            m = jnp.max(s, axis=-1, keepdims=True)
            p = jnp.exp(s - m)
            l = jnp.sum(p, axis=-1, keepdims=True)
            pb = p.astype(bf16)
            rl = 1.0 / l
            for part in range(HG // VP):
                wait_all(vbuf.at[j, :, pl.ds(part * VP, VP)], vsem.at[(g % 2) * (HG // VP) + part])
                if part == HG // VP - 1:
                    @pl.when((g == 1) | (g == 2))
                    def _():
                        start_v(j + 1)

                    @pl.when(g == 3)
                    def _():
                        start_v(j + 1, 2)
                o = None
                for c in range(NC):
                    d = jax.lax.dot_general(
                        pb[:, 128 * c:128 * (c + 1)],
                        _as_bf16(v32[j, c, pl.ds(part * VP, VP)].reshape(VP * DH2, 128)),
                        (((1,), (1,)), ((), ())), preferred_element_type=f32)
                    o = d if o is None else o + d
                cols = slice(part * VP * DH, (part + 1) * VP * DH)
                om = jnp.where(mask[:, cols], o * rl, 0.0).astype(bf16)
                acc = acc + wo_proj(om, pl.multiple_of(g * (GW // 2) + part * VP * DH2, 8), VP * DH2)
            return acc

        acc = jax.lax.fori_loop(0, NG, group, jnp.zeros((HG, D), f32))
        return x + jnp.broadcast_to(jnp.sum(acc, axis=0, keepdims=True), (HG, D))

    lane = jax.lax.broadcasted_iota(jnp.int32, (HG, 128), 1)
    sub = jax.lax.broadcasted_iota(jnp.int32, (HG, 128), 0)
    dl = lane - 2 * sub

    def attention2(x, b):
        h = _ln(x).astype(bf16)
        st = {'acc': None}

        def tile_mask(t):
            c = lane + 128 * t
            return (c >= sub * DH) & (c < sub * DH + DH)

        def q_tile(u):
            q = _mm(h, _as_bf16(wq32[u]))
            st['q', u] = jnp.where(tile_mask(u % UT), q, 0.0).astype(bf16)

        def k_rows(c, u):
            hd, r0 = divmod(64 * u, DH2)
            g, h0 = divmod(hd, HG)
            j = b * NG + g
            if r0 + 64 <= DH2:
                return k32[j, c, h0, pl.ds(r0, 64), :]
            return jnp.concatenate([k32[j, c, h0, pl.ds(r0, DH2 - r0), :],
                                    k32[j, c, h0 + 1, pl.ds(0, 64 - (DH2 - r0)), :]], axis=0)

        def s_tile(u):
            k, t = divmod(u, UT)
            qt = st.pop(('q', u))
            d = jnp.concatenate([_mm(qt, _as_bf16(k_rows(c, u))) for c in range(NC)], axis=1)
            st['s', k] = d if t == 0 else st['s', k] + d
            if t == UT - 1:
                sa = st.pop(('s', k))
                m = jnp.max(sa, axis=-1, keepdims=True)
                p = jnp.exp2((sa - m) * (SCALE * LOG2E))
                st['p', k] = p
                st['rl', k] = 1.0 / jnp.sum(p, axis=-1, keepdims=True)

        def v_tile(u):
            p = st['p', u // UT]
            tile = jnp.zeros((HG, 128), f32)
            for c in range(128 * u, 128 * u + 128, 16):
                hd, r = c // DH, (c % DH) // 16
                g, hh = divmod(hd, HG)
                if ('pb', hd) not in st:
                    hu = hd % U
                    st['pb', hd] = [jnp.broadcast_to(p[hu:hu + 1, 128 * i:128 * (i + 1)], (HG, 128))
                                    for i in range(NC)]
                pb = st['pb', hd]
                acc = []
                for half in range(2):
                    alo = ahi = None
                    for i in range(4 * half, 4 * half + 4):
                        w = v32[b * NG + g, i, hh, pl.ds(8 * r, 8), :]
                        lo = pltpu.bitcast(w << 16, f32) * pb[i]
                        hi = pltpu.bitcast(w & jnp.uint32(0xFFFF0000), f32) * pb[i]
                        alo = lo if alo is None else alo + lo
                        ahi = hi if ahi is None else ahi + hi
                    acc.append((alo, ahi))
                rlo = jnp.sum(acc[0][0], axis=-1, keepdims=True) + jnp.sum(acc[1][0], axis=-1, keepdims=True)
                rhi = jnp.sum(acc[0][1], axis=-1, keepdims=True) + jnp.sum(acc[1][1], axis=-1, keepdims=True)
                base = c % 128
                tile = jnp.where(dl == base, rlo, jnp.where(dl == base + 1, rhi, tile))

            def fac(hd):
                if ('f', hd) not in st:
                    st['f', hd] = jnp.broadcast_to(st['rl', hd // U][hd % U:hd % U + 1, :], (HG, 128))
                return st['f', hd]

            ha, hb = (128 * u) // DH, (128 * u + 127) // DH
            f = fac(ha) if ha == hb else jnp.where(lane < hb * DH - 128 * u, fac(ha), fac(hb))
            st['t', u] = (tile * f).astype(bf16)

        def w_tile(u):
            d = wo_proj(st.pop(('t', u)), 64 * u, 64)
            st['acc'] = d if st['acc'] is None else st['acc'] + d

        N = NG * NT
        SL = SLEAD * UT
        for m in range(-SL - QLEAD, N + WLAG):
            if 0 <= m + SL + QLEAD < N:
                q_tile(m + SL + QLEAD)
            if 0 <= m + SL < N:
                s_tile(m + SL)
            if 0 <= m < N:
                v_tile(m)
            if 0 <= m - WLAG < N:
                w_tile(m - WLAG)
        acc = st['acc']
        return x + jnp.broadcast_to(jnp.sum(acc, axis=0, keepdims=True), (HG, D))

    def ffn(x):
        h = _ln(x)
        r = jnp.sum(h * wr_row, axis=-1, keepdims=True)
        hb = h.astype(bf16)
        g = jnp.concatenate([_mm(hb, _as_bf16(wg32[t])) for t in range(NF)], axis=1)
        u = jnp.concatenate([_mm(hb, _as_bf16(wu32[t])) for t in range(NF)], axis=1)
        a = (g * jax.nn.sigmoid(g) * u).astype(bf16)
        y = jnp.concatenate([_mm(a, _as_bf16(wd32[n])) for n in range(ND)], axis=1)
        return x + h + y * jax.nn.sigmoid(r)

    def batch(b, out):
        xb = jnp.sum(jnp.where(row4 == b, x_all, 0.0), axis=0, keepdims=True)
        x = jnp.broadcast_to(xb, (HG, D))
        x = attention1(x, b)
        x = ffn(x)
        start_k(b * NG + 5, 2)
        x = attention2(x, b)
        start_v(b * NG + 5, 2)
        x = ffn(x)
        return jnp.where(row4 == b, x[:B, :], out)

    out = jax.lax.fori_loop(0, B - 1, batch, jnp.zeros((B, D), f32))
    out = batch(B - 1, out)
    o_ref[...] = out.astype(o_ref.dtype)


@jax.jit
def pallas_interleave_layers__sliding_block_cached__moe_arch_mod__decode_kernel(
    A_x: jax.Array,
    A_k_cache: jax.Array,
    A_v_cache: jax.Array,
    A_wq: jax.Array,
    A_wo: jax.Array,
    B_x: jax.Array,
    B_w_r: jax.Array,
    B_w_gate: jax.Array,
    B_w_up: jax.Array,
    B_w_down: jax.Array,
):
    del B_x
    k_t = jnp.transpose(A_k_cache, (0, 1, 3, 2))
    v_t = jnp.transpose(A_v_cache, (0, 1, 3, 2))
    any_spec = pl.BlockSpec(memory_space=pl.ANY)
    out = pl.pallas_call(
        _kernel,
        out_shape=jax.ShapeDtypeStruct((B, D), A_x.dtype),
        in_specs=[any_spec] * 9,
        out_specs=pl.BlockSpec(memory_space=pltpu.VMEM),
        scratch_shapes=[
            pltpu.VMEM((NJ, NC, HG, DH, 128), bf16),
            pltpu.VMEM((NJ, NC, HG, DH, 128), bf16),
            pltpu.VMEM((H * DH // 128, D, 128), bf16),
            pltpu.VMEM((ND, H * DH, 128), bf16),
            pltpu.VMEM((NF, D, 128), bf16),
            pltpu.VMEM((NF, D, 128), bf16),
            pltpu.VMEM((ND, F, 128), bf16),
            pltpu.VMEM((B, D), bf16),
            pltpu.VMEM((ND, 128), bf16),
            pltpu.SemaphoreType.DMA((2,)),
            pltpu.SemaphoreType.DMA((2 * HG // VP,)),
            pltpu.SemaphoreType.DMA(()),
        ],
        compiler_params=pltpu.CompilerParams(vmem_limit_bytes=126 * 1024 * 1024),
    )(A_x.reshape(B, D), B_w_r.reshape(ND, 128), k_t, v_t,
      A_wq, A_wo, B_w_gate, B_w_up, B_w_down)
    return out.reshape(B, 1, D)
```

```python
import jax
import jax.numpy as jnp
from jax.experimental import pallas as pl
from jax.experimental.pallas import tpu as pltpu

B, D, H, DH, SK, F = 4, 640, 32, 192, 4096, 1536
W = min(4096, max(256, SK // 4))
HG = 8
NG = H // HG
NJ = B * NG
GW = HG * DH
DH2 = DH // 2
NC = W // 128
NT = GW // 128
ND = D // 128
NF = F // 128
EPS = 1e-5
SCALE = DH ** -0.5
LOG2E = 1.4426950408889634
VP = 2
U = 4
UT = U * DH // 128
SLEAD = 2
QLEAD = 2
WLAG = 24
MFEED = 16

f32, bf16, u32 = jnp.float32, jnp.bfloat16, jnp.uint32


def _ln(x):
    m = jnp.mean(x, axis=-1, keepdims=True)
    m2 = jnp.mean(x * x, axis=-1, keepdims=True)
    v = jnp.maximum(m2 - m * m, 0.0)
    return (x - m) * jax.lax.rsqrt(v + EPS)


def _as_bf16(w):
    return pltpu.bitcast(w, bf16)


def _mm(a, w):
    return jnp.dot(a, w, preferred_element_type=f32)


def _kernel(x_hbm, wr_hbm, k_hbm, v_hbm, wq_hbm, wo_hbm, wg_hbm, wu_hbm, wd_hbm,
            o_ref,
            kbuf, vbuf, wq_b, wo_b, wg_b, wu_b, wd_b, x_s, wr_s,
            ksem, vsem, wsem):
    k32, v32 = kbuf.bitcast(u32), vbuf.bitcast(u32)
    wq32, wo32 = wq_b.bitcast(u32), wo_b.bitcast(u32)
    wg32, wu32, wd32 = wg_b.bitcast(u32), wu_b.bitcast(u32), wd_b.bitcast(u32)

    def start_kv(src, dst, sems, j, hp, sem_heads, ring):
        b = j // NG
        g = j % NG

        def heads(i, carry):
            sem = sems.at[(j % ring) * (HG // sem_heads) + (i * hp) // sem_heads]
            for c in range(NC):
                pltpu.make_async_copy(
                    src.at[b, pl.ds(g * HG + i * hp, hp), :, pl.ds(SK - W + c * 128, 128)],
                    dst.at[j, c, pl.ds(i * hp, hp)],
                    sem).start(priority=c % 2)
            return carry

        jax.lax.fori_loop(0, HG // hp, heads, 0)

    def start_k(j, hp=1):
        if isinstance(j, int):
            if j < NJ:
                start_kv(k_hbm, kbuf, ksem, j, hp, HG, NG)
            return

        @pl.when(j < NJ)
        def _():
            start_kv(k_hbm, kbuf, ksem, j, hp, HG, NG)

    def start_v(j, hp=1):
        if isinstance(j, int):
            if j < NJ:
                start_kv(v_hbm, vbuf, vsem, j, hp, VP, 2)
            return

        @pl.when(j < NJ)
        def _():
            start_kv(v_hbm, vbuf, vsem, j, hp, VP, 2)

    def wait_all(buf, sem):
        pltpu.make_async_copy(buf, buf, sem).wait()

    def start_w(src, dst, sem, rp):
        rows, cols = src.shape
        n = 0
        for r in range(rows // rp):
            for c in range(cols // 128):
                pltpu.make_async_copy(src.at[pl.ds(r * rp, rp), pl.ds(c * 128, 128)],
                                      dst.at[c, pl.ds(r * rp, rp), :],
                                      sem).start(priority=n % 2)
                n += 1

    pltpu.make_async_copy(x_hbm, x_s, wsem).start()
    pltpu.make_async_copy(wr_hbm, wr_s, wsem).start()
    start_w(wq_hbm, wq_b, wsem, 320)
    start_w(wo_hbm, wo_b, wsem, 96)
    start_w(wg_hbm, wg_b, wsem, 320)
    start_w(wu_hbm, wu_b, wsem, 320)
    start_w(wd_hbm, wd_b, wsem, 96)
    start_k(0)
    start_v(0)
    start_k(1)
    start_v(1)
    start_k(2)

    for buf in (x_s, wr_s, wq_b, wo_b, wg_b, wu_b, wd_b):
        wait_all(buf, wsem)
    x_all = x_s[...].astype(f32)
    wr = wr_s[...].astype(f32)
    wr_row = jnp.concatenate([wr[i:i + 1, :] for i in range(ND)], axis=1)

    row = jax.lax.broadcasted_iota(jnp.int32, (HG, GW), 0)
    col = jax.lax.broadcasted_iota(jnp.int32, (HG, GW), 1)
    mask = (col >= row * DH) & (col < row * DH + DH)
    row4 = jax.lax.broadcasted_iota(jnp.int32, (B, D), 0)

    def wo_proj(t, r0, nr):
        return jnp.concatenate(
            [_mm(t, _as_bf16(wo32[n, pl.ds(r0, nr), :])) for n in range(ND)], axis=1)

    def attention1(x, b):
        h = _ln(x).astype(bf16)

        def group(g, acc):
            j = b * NG + g
            q = jnp.concatenate(
                [_mm(h, _as_bf16(wq32[g * NT + t])) for t in range(NT)], axis=1)
            qbd = jnp.where(mask, q, 0.0).astype(bf16)
            wait_all(kbuf.at[j], ksem.at[g])

            @pl.when(g == 3)
            def _():
                start_k(j + 1)
            s = jnp.concatenate(
                [_mm(qbd, _as_bf16(k32[j, c].reshape(HG * DH2, 128))) for c in range(NC)],
                axis=1) * SCALE
            m = jnp.max(s, axis=-1, keepdims=True)
            p = jnp.exp(s - m)
            l = jnp.sum(p, axis=-1, keepdims=True)
            pb = p.astype(bf16)
            rl = 1.0 / l
            for part in range(HG // VP):
                wait_all(vbuf.at[j, :, pl.ds(part * VP, VP)], vsem.at[(g % 2) * (HG // VP) + part])
                if part == HG // VP - 1:
                    @pl.when(g == 3)
                    def _():
                        start_v(j + 1)
                o = None
                for c in range(NC):
                    d = jax.lax.dot_general(
                        pb[:, 128 * c:128 * (c + 1)],
                        _as_bf16(v32[j, c, pl.ds(part * VP, VP)].reshape(VP * DH2, 128)),
                        (((1,), (1,)), ((), ())), preferred_element_type=f32)
                    o = d if o is None else o + d
                cols = slice(part * VP * DH, (part + 1) * VP * DH)
                om = jnp.where(mask[:, cols], o * rl, 0.0).astype(bf16)
                acc = acc + wo_proj(om, pl.multiple_of(g * (GW // 2) + part * VP * DH2, 8), VP * DH2)

            @pl.when((g == 0) | (g == 2))
            def _():
                start_v(j + 2 - g // 2)

            @pl.when(g == 1)
            def _():
                start_k(j + 2)
            return acc

        acc = jax.lax.fori_loop(0, NG, group, jnp.zeros((HG, D), f32))
        return x + jnp.broadcast_to(jnp.sum(acc, axis=0, keepdims=True), (HG, D))

    lane = jax.lax.broadcasted_iota(jnp.int32, (HG, 128), 1)
    sub = jax.lax.broadcasted_iota(jnp.int32, (HG, 128), 0)
    dl = lane - 2 * sub

    def attention2(x, b, feed):
        h = _ln(x).astype(bf16)
        st = {'acc': None}

        def tile_mask(t):
            c = lane + 128 * t
            return (c >= sub * DH) & (c < sub * DH + DH)

        def q_tile(u):
            q = _mm(h, _as_bf16(wq32[u]))
            st['q', u] = jnp.where(tile_mask(u % UT), q, 0.0).astype(bf16)

        def k_rows(c, u):
            hd, r0 = divmod(64 * u, DH2)
            g, h0 = divmod(hd, HG)
            j = b * NG + g
            if r0 + 64 <= DH2:
                return k32[j, c, h0, pl.ds(r0, 64), :]
            return jnp.concatenate([k32[j, c, h0, pl.ds(r0, DH2 - r0), :],
                                    k32[j, c, h0 + 1, pl.ds(0, 64 - (DH2 - r0)), :]], axis=0)

        def s_tile(u):
            k, t = divmod(u, UT)
            qt = st.pop(('q', u))
            d = jnp.concatenate([_mm(qt, _as_bf16(k_rows(c, u))) for c in range(NC)], axis=1)
            st['s', k] = d if t == 0 else st['s', k] + d
            if t == UT - 1:
                sa = st.pop(('s', k))
                m = jnp.max(sa, axis=-1, keepdims=True)
                p = jnp.exp2((sa - m) * (SCALE * LOG2E))
                st['p', k] = p
                st['rl', k] = 1.0 / jnp.sum(p, axis=-1, keepdims=True)

        def v_tile(u):
            p = st['p', u // UT]
            tile = jnp.zeros((HG, 128), f32)
            for c in range(128 * u, 128 * u + 128, 16):
                hd, r = c // DH, (c % DH) // 16
                g, hh = divmod(hd, HG)
                if ('pb', hd) not in st:
                    hu = hd % U
                    st['pb', hd] = [jnp.broadcast_to(p[hu:hu + 1, 128 * i:128 * (i + 1)], (HG, 128))
                                    for i in range(NC)]
                pb = st['pb', hd]
                acc = []
                for half in range(2):
                    alo = ahi = None
                    for i in range(4 * half, 4 * half + 4):
                        w = v32[b * NG + g, i, hh, pl.ds(8 * r, 8), :]
                        lo = pltpu.bitcast(w << 16, f32) * pb[i]
                        hi = pltpu.bitcast(w & jnp.uint32(0xFFFF0000), f32) * pb[i]
                        alo = lo if alo is None else alo + lo
                        ahi = hi if ahi is None else ahi + hi
                    acc.append((alo, ahi))
                rlo = jnp.sum(acc[0][0], axis=-1, keepdims=True) + jnp.sum(acc[1][0], axis=-1, keepdims=True)
                rhi = jnp.sum(acc[0][1], axis=-1, keepdims=True) + jnp.sum(acc[1][1], axis=-1, keepdims=True)
                base = c % 128
                tile = jnp.where(dl == base, rlo, jnp.where(dl == base + 1, rhi, tile))

            def fac(hd):
                if ('f', hd) not in st:
                    st['f', hd] = jnp.broadcast_to(st['rl', hd // U][hd % U:hd % U + 1, :], (HG, 128))
                return st['f', hd]

            ha, hb = (128 * u) // DH, (128 * u + 127) // DH
            f = fac(ha) if ha == hb else jnp.where(lane < hb * DH - 128 * u, fac(ha), fac(hb))
            st['t', u] = (tile * f).astype(bf16)

        def w_tile(u):
            d = wo_proj(st.pop(('t', u)), 64 * u, 64)
            st['acc'] = d if st['acc'] is None else st['acc'] + d

        N = NG * NT
        SL = SLEAD * UT
        for m in range(-SL - QLEAD, N + WLAG):
            if m == MFEED:
                feed()
            if 0 <= m + SL + QLEAD < N:
                q_tile(m + SL + QLEAD)
            if 0 <= m + SL < N:
                s_tile(m + SL)
            if 0 <= m < N:
                v_tile(m)
            if 0 <= m - WLAG < N:
                w_tile(m - WLAG)
        acc = st['acc']
        return x + jnp.broadcast_to(jnp.sum(acc, axis=0, keepdims=True), (HG, D))

    def ffn(x):
        h = _ln(x)
        r = jnp.sum(h * wr_row, axis=-1, keepdims=True)
        hb = h.astype(bf16)
        g = jnp.concatenate([_mm(hb, _as_bf16(wg32[t])) for t in range(NF)], axis=1)
        u = jnp.concatenate([_mm(hb, _as_bf16(wu32[t])) for t in range(NF)], axis=1)
        a = (g * jax.nn.sigmoid(g) * u).astype(bf16)
        y = jnp.concatenate([_mm(a, _as_bf16(wd32[n])) for n in range(ND)], axis=1)
        return x + h + y * jax.nn.sigmoid(r)

    def batch(b, out):
        xb = jnp.sum(jnp.where(row4 == b, x_all, 0.0), axis=0, keepdims=True)
        x = jnp.broadcast_to(xb, (HG, D))
        x = attention1(x, b)
        x = ffn(x)
        start_k(b * NG + 5)
        x = attention2(x, b, lambda: start_v(b * NG + 5))
        start_k(b * NG + 6)
        x = ffn(x)
        return jnp.where(row4 == b, x[:B, :], out)

    out = jax.lax.fori_loop(0, B - 1, batch, jnp.zeros((B, D), f32))
    out = batch(B - 1, out)
    o_ref[...] = out.astype(o_ref.dtype)


@jax.jit
def pallas_interleave_layers__sliding_block_cached__moe_arch_mod__decode_kernel(
    A_x: jax.Array,
    A_k_cache: jax.Array,
    A_v_cache: jax.Array,
    A_wq: jax.Array,
    A_wo: jax.Array,
    B_x: jax.Array,
    B_w_r: jax.Array,
    B_w_gate: jax.Array,
    B_w_up: jax.Array,
    B_w_down: jax.Array,
):
    del B_x
    k_t = jnp.transpose(A_k_cache, (0, 1, 3, 2))
    v_t = jnp.transpose(A_v_cache, (0, 1, 3, 2))
    any_spec = pl.BlockSpec(memory_space=pl.ANY)
    out = pl.pallas_call(
        _kernel,
        out_shape=jax.ShapeDtypeStruct((B, D), A_x.dtype),
        in_specs=[any_spec] * 9,
        out_specs=pl.BlockSpec(memory_space=pltpu.VMEM),
        scratch_shapes=[
            pltpu.VMEM((NJ, NC, HG, DH, 128), bf16),
            pltpu.VMEM((NJ, NC, HG, DH, 128), bf16),
            pltpu.VMEM((H * DH // 128, D, 128), bf16),
            pltpu.VMEM((ND, H * DH, 128), bf16),
            pltpu.VMEM((NF, D, 128), bf16),
            pltpu.VMEM((NF, D, 128), bf16),
            pltpu.VMEM((ND, F, 128), bf16),
            pltpu.VMEM((B, D), bf16),
            pltpu.VMEM((ND, 128), bf16),
            pltpu.SemaphoreType.DMA((NG,)),
            pltpu.SemaphoreType.DMA((2 * HG // VP,)),
            pltpu.SemaphoreType.DMA(()),
        ],
        compiler_params=pltpu.CompilerParams(vmem_limit_bytes=126 * 1024 * 1024),
    )(A_x.reshape(B, D), B_w_r.reshape(ND, 128), k_t, v_t,
      A_wq, A_wo, B_w_gate, B_w_up, B_w_down)
    return out.reshape(B, 1, D)
```

```python
import jax
import jax.numpy as jnp
from jax.experimental import pallas as pl
from jax.experimental.pallas import tpu as pltpu

B, D, H, DH, SK, F = 4, 640, 32, 192, 4096, 1536
W = min(4096, max(256, SK // 4))
HG = 8
NG = H // HG
NJ = B * NG
GW = HG * DH
DH2 = DH // 2
NC = W // 128
NT = GW // 128
ND = D // 128
NF = F // 128
EPS = 1e-5
SCALE = DH ** -0.5
LOG2E = 1.4426950408889634
VP = 2
U = 4
UT = U * DH // 128
SLEAD = 2
QLEAD = 2
WLAG = 24
MFEED = 16
NV, DV = 3, 4

f32, bf16, u32 = jnp.float32, jnp.bfloat16, jnp.uint32


def _ln(x):
    m = jnp.mean(x, axis=-1, keepdims=True)
    m2 = jnp.mean(x * x, axis=-1, keepdims=True)
    v = jnp.maximum(m2 - m * m, 0.0)
    return (x - m) * jax.lax.rsqrt(v + EPS)


def _as_bf16(w):
    return pltpu.bitcast(w, bf16)


def _lo(w):
    return pltpu.bitcast(w << 16, f32)


def _hi(w):
    return pltpu.bitcast(w & jnp.uint32(0xFFFF0000), f32)


def _mm(a, w):
    return jnp.dot(a, w, preferred_element_type=f32)


def _kernel(x_hbm, wr_hbm, k_hbm, v_hbm, wq_hbm, wo_hbm, wg_hbm, wu_hbm, wd_hbm,
            o_ref,
            kbuf, vbuf, wq_b, wo_b, wg_b, wu_b, wd_b, x_s, wr_s,
            ksem, vsem, wsem):
    k32, v32 = kbuf.bitcast(u32), vbuf.bitcast(u32)
    wq32, wo32 = wq_b.bitcast(u32), wo_b.bitcast(u32)
    wg32, wu32, wd32 = wg_b.bitcast(u32), wu_b.bitcast(u32), wd_b.bitcast(u32)

    def start_kv(src, dst, sems, j, hp, sem_heads, ring):
        b = j // NG
        g = j % NG

        def heads(i, carry):
            sem = sems.at[(j % ring) * (HG // sem_heads) + (i * hp) // sem_heads]
            for c in range(NC):
                pltpu.make_async_copy(
                    src.at[b, pl.ds(g * HG + i * hp, hp), :, pl.ds(SK - W + c * 128, 128)],
                    dst.at[j, c, pl.ds(i * hp, hp)],
                    sem).start(priority=c % 2)
            return carry

        jax.lax.fori_loop(0, HG // hp, heads, 0)

    def start_k(j, hp=1):
        if isinstance(j, int):
            if j < NJ:
                start_kv(k_hbm, kbuf, ksem, j, hp, HG, NG)
            return

        @pl.when(j < NJ)
        def _():
            start_kv(k_hbm, kbuf, ksem, j, hp, HG, NG)

    def start_v(j, hp=1):
        if isinstance(j, int):
            if j < NJ:
                start_kv(v_hbm, vbuf, vsem, j, hp, VP, 2)
            return

        @pl.when(j < NJ)
        def _():
            start_kv(v_hbm, vbuf, vsem, j, hp, VP, 2)

    def wait_all(buf, sem):
        pltpu.make_async_copy(buf, buf, sem).wait()

    def start_w(src, dst, sem, rp):
        rows, cols = src.shape
        n = 0
        for r in range(rows // rp):
            for c in range(cols // 128):
                pltpu.make_async_copy(src.at[pl.ds(r * rp, rp), pl.ds(c * 128, 128)],
                                      dst.at[c, pl.ds(r * rp, rp), :],
                                      sem).start(priority=n % 2)
                n += 1

    pltpu.make_async_copy(x_hbm, x_s, wsem).start()
    pltpu.make_async_copy(wr_hbm, wr_s, wsem).start()
    start_w(wq_hbm, wq_b, wsem, 320)
    start_w(wo_hbm, wo_b, wsem, 96)
    start_w(wg_hbm, wg_b, wsem, 320)
    start_w(wu_hbm, wu_b, wsem, 320)
    start_w(wd_hbm, wd_b, wsem, 96)
    start_k(0)
    start_v(0)
    start_k(1)
    start_v(1)
    start_k(2)

    for buf in (x_s, wr_s, wq_b, wo_b, wg_b, wu_b, wd_b):
        wait_all(buf, wsem)
    x_all = x_s[...].astype(f32)
    wr = wr_s[...].astype(f32)
    wr_row = jnp.concatenate([wr[i:i + 1, :] for i in range(ND)], axis=1)

    row = jax.lax.broadcasted_iota(jnp.int32, (HG, GW), 0)
    col = jax.lax.broadcasted_iota(jnp.int32, (HG, GW), 1)
    mask = (col >= row * DH) & (col < row * DH + DH)
    row4 = jax.lax.broadcasted_iota(jnp.int32, (B, D), 0)

    def wo_proj(t, r0, nr):
        return jnp.concatenate(
            [_mm(t, _as_bf16(wo32[n, pl.ds(r0, nr), :])) for n in range(ND)], axis=1)

    def attention1(x, b):
        h = _ln(x).astype(bf16)

        def group(g, acc):
            j = b * NG + g
            q = jnp.concatenate(
                [_mm(h, _as_bf16(wq32[g * NT + t])) for t in range(NT)], axis=1)
            qbd = jnp.where(mask, q, 0.0).astype(bf16)
            wait_all(kbuf.at[j], ksem.at[g])

            @pl.when(g == 3)
            def _():
                start_k(j + 1)
            s = jnp.concatenate(
                [_mm(qbd, _as_bf16(k32[j, c].reshape(HG * DH2, 128))) for c in range(NC)],
                axis=1) * SCALE
            m = jnp.max(s, axis=-1, keepdims=True)
            p = jnp.exp(s - m)
            l = jnp.sum(p, axis=-1, keepdims=True)
            pb = p.astype(bf16)
            rl = 1.0 / l
            for part in range(HG // VP):
                wait_all(vbuf.at[j, :, pl.ds(part * VP, VP)], vsem.at[(g % 2) * (HG // VP) + part])
                if part == HG // VP - 1:
                    @pl.when(g == 3)
                    def _():
                        start_v(j + 1)
                o = None
                for c in range(NC):
                    d = jax.lax.dot_general(
                        pb[:, 128 * c:128 * (c + 1)],
                        _as_bf16(v32[j, c, pl.ds(part * VP, VP)].reshape(VP * DH2, 128)),
                        (((1,), (1,)), ((), ())), preferred_element_type=f32)
                    o = d if o is None else o + d
                cols = slice(part * VP * DH, (part + 1) * VP * DH)
                om = jnp.where(mask[:, cols], o * rl, 0.0).astype(bf16)
                acc = acc + wo_proj(om, pl.multiple_of(g * (GW // 2) + part * VP * DH2, 8), VP * DH2)

            @pl.when((g == 0) | (g == 2))
            def _():
                start_v(j + 2 - g // 2)

            @pl.when(g == 1)
            def _():
                start_k(j + 2)
            return acc

        acc = jax.lax.fori_loop(0, NG, group, jnp.zeros((HG, D), f32))
        return x + jnp.broadcast_to(jnp.sum(acc, axis=0, keepdims=True), (HG, D))

    lane = jax.lax.broadcasted_iota(jnp.int32, (HG, 128), 1)
    sub = jax.lax.broadcasted_iota(jnp.int32, (HG, 128), 0)
    dl = lane - 2 * sub

    def attention2(x, b, feed):
        h = _ln(x).astype(bf16)
        st = {'acc': None}

        def tile_mask(t):
            c = lane + 128 * t
            return (c >= sub * DH) & (c < sub * DH + DH)

        def q_tile(u):
            q = _mm(h, _as_bf16(wq32[u]))
            st['q', u] = jnp.where(tile_mask(u % UT), q, 0.0).astype(bf16)

        def k_rows(c, u):
            hd, r0 = divmod(64 * u, DH2)
            g, h0 = divmod(hd, HG)
            j = b * NG + g
            if r0 + 64 <= DH2:
                return k32[j, c, h0, pl.ds(r0, 64), :]
            return jnp.concatenate([k32[j, c, h0, pl.ds(r0, DH2 - r0), :],
                                    k32[j, c, h0 + 1, pl.ds(0, 64 - (DH2 - r0)), :]], axis=0)

        def s_tile(u):
            k, t = divmod(u, UT)
            qt = st.pop(('q', u))
            d = jnp.concatenate([_mm(qt, _as_bf16(k_rows(c, u))) for c in range(NC)], axis=1)
            st['s', k] = d if t == 0 else st['s', k] + d
            if t == UT - 1:
                sa = st.pop(('s', k))
                m = jnp.max(sa, axis=-1, keepdims=True)
                p = jnp.exp2((sa - m) * (SCALE * LOG2E))
                st['p', k] = p
                st['rl', k] = 1.0 / jnp.sum(p, axis=-1, keepdims=True)

        def v_tile(u):
            p = st['p', u // UT]
            tile = jnp.zeros((HG, 128), f32)
            for c in range(128 * u, 128 * u + 128, 16):
                hd, r = c // DH, (c % DH) // 16
                g, hh = divmod(hd, HG)
                if ('pb', hd) not in st:
                    hu = hd % U
                    st['pb', hd] = [jnp.broadcast_to(p[hu:hu + 1, 128 * i:128 * (i + 1)], (HG, 128))
                                    for i in range(NC)]
                pb = st['pb', hd]
                acc = []
                for half in range(2):
                    alo = ahi = None
                    for i in range(4 * half, 4 * half + 4):
                        w = v32[b * NG + g, i, hh, pl.ds(8 * r, 8), :]
                        lo = _lo(w) * pb[i]
                        hi = _hi(w) * pb[i]
                        alo = lo if alo is None else alo + lo
                        ahi = hi if ahi is None else ahi + hi
                    acc.append((alo, ahi))
                rlo = jnp.sum(acc[0][0], axis=-1, keepdims=True) + jnp.sum(acc[1][0], axis=-1, keepdims=True)
                rhi = jnp.sum(acc[0][1], axis=-1, keepdims=True) + jnp.sum(acc[1][1], axis=-1, keepdims=True)
                base = c % 128
                tile = jnp.where(dl == base, rlo, jnp.where(dl == base + 1, rhi, tile))

            def fac(hd):
                if ('f', hd) not in st:
                    st['f', hd] = jnp.broadcast_to(st['rl', hd // U][hd % U:hd % U + 1, :], (HG, 128))
                return st['f', hd]

            ha, hb = (128 * u) // DH, (128 * u + 127) // DH
            f = fac(ha) if ha == hb else jnp.where(lane < hb * DH - 128 * u, fac(ha), fac(hb))
            st['t', u] = (tile * f).astype(bf16)

        def w_tile(u):
            d = wo_proj(st.pop(('t', u)), 64 * u, 64)
            st['acc'] = d if st['acc'] is None else st['acc'] + d

        N = NG * NT
        SL = SLEAD * UT
        for m in range(-SL - QLEAD, N + WLAG):
            if m == MFEED:
                feed()
            if 0 <= m + SL + QLEAD < N:
                q_tile(m + SL + QLEAD)
            if 0 <= m + SL < N:
                s_tile(m + SL)
            if 0 <= m < N:
                v_tile(m)
            if 0 <= m - WLAG < N:
                w_tile(m - WLAG)
        acc = st['acc']
        return x + jnp.broadcast_to(jnp.sum(acc, axis=0, keepdims=True), (HG, D))

    def spread(v, rblk):
        t, base = divmod(16 * rblk, 128)
        vt = v[:, 128 * t:128 * (t + 1)]
        even = jnp.sum(jnp.where(dl == base, vt, 0.0), axis=-1, keepdims=True)
        odd = jnp.sum(jnp.where(dl == base + 1, vt, 0.0), axis=-1, keepdims=True)
        return even, odd

    def rowsum(a):
        return jnp.broadcast_to(jnp.sum(a, axis=0, keepdims=True), a.shape)

    def ffn(x):
        h = _ln(x)
        r = jnp.sum(h * wr_row, axis=-1, keepdims=True)
        hb = h.astype(bf16)
        a = [None] * NF
        accs = {}
        gate = [None]

        def act(g, u):
            return (g * jax.nn.sigmoid(g) * u).astype(bf16)

        def vpu_blocks():
            hr = hb.astype(f32)
            for rb in range(D // 16):
                even, odd = spread(hr, rb)
                if gate[0] is not None:
                    even = even + gate[0]
                for t in range(NF - NV, NF):
                    for nm, w32 in (('g', wg32), ('u', wu32)):
                        w = w32[t, pl.ds(8 * rb, 8), :]
                        d = _lo(w) * even + _hi(w) * odd
                        accs[nm, t] = d if rb == 0 else accs[nm, t] + d
                yield

        blocks = vpu_blocks()
        per = -(-(D // 16) // (NF - NV))
        for t in range(NF - NV):
            for _ in range(per):
                next(blocks, None)
            g = _mm(hb, _as_bf16(wg32[t]))
            u = _mm(hb, _as_bf16(wu32[t]))
            gate[0] = g * 0.0
            a[t] = act(g, u)
        for _ in blocks:
            pass
        for t in range(NF - NV, NF):
            a[t] = act(rowsum(accs['g', t]), rowsum(accs['u', t]))
        nk = NF - DV
        am = jnp.concatenate(a[:nk], axis=1)
        y = [_mm(am, _as_bf16(wd32[n, pl.ds(0, 64 * nk), :])) for n in range(ND)]
        yv = [None] * ND
        for t in range(nk, NF):
            af = a[t].astype(f32)
            for rb in range(8):
                even, odd = spread(af, rb)
                for n in range(ND):
                    w = wd32[n, pl.ds(64 * t + 8 * rb, 8), :]
                    d = _lo(w) * even + _hi(w) * odd
                    yv[n] = d if yv[n] is None else yv[n] + d
        y = jnp.concatenate([y[n] + rowsum(yv[n]) for n in range(ND)], axis=1)
        return x + h + y * jax.nn.sigmoid(r)

    def batch(b, out):
        xb = jnp.sum(jnp.where(row4 == b, x_all, 0.0), axis=0, keepdims=True)
        x = jnp.broadcast_to(xb, (HG, D))
        x = attention1(x, b)
        x = ffn(x)
        start_k(b * NG + 5)
        x = attention2(x, b, lambda: start_v(b * NG + 5))
        start_k(b * NG + 6)
        x = ffn(x)
        return jnp.where(row4 == b, x[:B, :], out)

    out = jax.lax.fori_loop(0, B - 1, batch, jnp.zeros((B, D), f32))
    out = batch(B - 1, out)
    o_ref[...] = out.astype(o_ref.dtype)


@jax.jit
def pallas_interleave_layers__sliding_block_cached__moe_arch_mod__decode_kernel(
    A_x: jax.Array,
    A_k_cache: jax.Array,
    A_v_cache: jax.Array,
    A_wq: jax.Array,
    A_wo: jax.Array,
    B_x: jax.Array,
    B_w_r: jax.Array,
    B_w_gate: jax.Array,
    B_w_up: jax.Array,
    B_w_down: jax.Array,
):
    del B_x
    k_t = jnp.transpose(A_k_cache, (0, 1, 3, 2))
    v_t = jnp.transpose(A_v_cache, (0, 1, 3, 2))
    any_spec = pl.BlockSpec(memory_space=pl.ANY)
    out = pl.pallas_call(
        _kernel,
        out_shape=jax.ShapeDtypeStruct((B, D), A_x.dtype),
        in_specs=[any_spec] * 9,
        out_specs=pl.BlockSpec(memory_space=pltpu.VMEM),
        scratch_shapes=[
            pltpu.VMEM((NJ, NC, HG, DH, 128), bf16),
            pltpu.VMEM((NJ, NC, HG, DH, 128), bf16),
            pltpu.VMEM((H * DH // 128, D, 128), bf16),
            pltpu.VMEM((ND, H * DH, 128), bf16),
            pltpu.VMEM((NF, D, 128), bf16),
            pltpu.VMEM((NF, D, 128), bf16),
            pltpu.VMEM((ND, F, 128), bf16),
            pltpu.VMEM((B, D), bf16),
            pltpu.VMEM((ND, 128), bf16),
            pltpu.SemaphoreType.DMA((NG,)),
            pltpu.SemaphoreType.DMA((2 * HG // VP,)),
            pltpu.SemaphoreType.DMA(()),
        ],
        compiler_params=pltpu.CompilerParams(vmem_limit_bytes=126 * 1024 * 1024),
    )(A_x.reshape(B, D), B_w_r.reshape(ND, 128), k_t, v_t,
      A_wq, A_wo, B_w_gate, B_w_up, B_w_down)
    return out.reshape(B, 1, D)
```

```python
import jax
import jax.numpy as jnp
from jax.experimental import pallas as pl
from jax.experimental.pallas import tpu as pltpu

B, D, H, DH, SK, F = 4, 640, 32, 192, 4096, 1536
W = min(4096, max(256, SK // 4))
HG = 8
NG = H // HG
NJ = B * NG
GW = HG * DH
DH2 = DH // 2
NC = W // 128
NT = GW // 128
ND = D // 128
NF = F // 128
EPS = 1e-5
SCALE = DH ** -0.5
LOG2E = 1.4426950408889634
VP = 2
U = 4
UT = U * DH // 128
SLEAD = 2
QLEAD = 2
WLAG = 24
MFEED = 16
VQ, VQP = 4, 5
VWO = 46
NV, DV = 3, 4

f32, bf16, u32 = jnp.float32, jnp.bfloat16, jnp.uint32


def _ln(x):
    m = jnp.mean(x, axis=-1, keepdims=True)
    m2 = jnp.mean(x * x, axis=-1, keepdims=True)
    v = jnp.maximum(m2 - m * m, 0.0)
    return (x - m) * jax.lax.rsqrt(v + EPS)


def _as_bf16(w):
    return pltpu.bitcast(w, bf16)


def _lo(w):
    return pltpu.bitcast(w << 16, f32)


def _hi(w):
    return pltpu.bitcast(w & jnp.uint32(0xFFFF0000), f32)


def _mm(a, w):
    return jnp.dot(a, w, preferred_element_type=f32)


def _kernel(x_hbm, wr_hbm, k_hbm, v_hbm, wq_hbm, wo_hbm, wg_hbm, wu_hbm, wd_hbm,
            o_ref,
            kbuf, vbuf, wq_b, wo_b, wg_b, wu_b, wd_b, x_s, wr_s,
            ksem, vsem, wsem):
    k32, v32 = kbuf.bitcast(u32), vbuf.bitcast(u32)
    wq32, wo32 = wq_b.bitcast(u32), wo_b.bitcast(u32)
    wg32, wu32, wd32 = wg_b.bitcast(u32), wu_b.bitcast(u32), wd_b.bitcast(u32)

    def start_kv(src, dst, sems, j, hp, sem_heads, ring):
        b = j // NG
        g = j % NG

        def heads(i, carry):
            sem = sems.at[(j % ring) * (HG // sem_heads) + (i * hp) // sem_heads]
            for c in range(NC):
                pltpu.make_async_copy(
                    src.at[b, pl.ds(g * HG + i * hp, hp), :, pl.ds(SK - W + c * 128, 128)],
                    dst.at[j, c, pl.ds(i * hp, hp)],
                    sem).start(priority=c % 2)
            return carry

        jax.lax.fori_loop(0, HG // hp, heads, 0)

    def start_k(j, hp=1):
        if isinstance(j, int):
            if j < NJ:
                start_kv(k_hbm, kbuf, ksem, j, hp, HG, NG)
            return

        @pl.when(j < NJ)
        def _():
            start_kv(k_hbm, kbuf, ksem, j, hp, HG, NG)

    def start_v(j, hp=1):
        if isinstance(j, int):
            if j < NJ:
                start_kv(v_hbm, vbuf, vsem, j, hp, VP, 2)
            return

        @pl.when(j < NJ)
        def _():
            start_kv(v_hbm, vbuf, vsem, j, hp, VP, 2)

    def wait_all(buf, sem):
        pltpu.make_async_copy(buf, buf, sem).wait()

    def start_w(src, dst, sem, rp):
        rows, cols = src.shape
        n = 0
        for r in range(rows // rp):
            for c in range(cols // 128):
                pltpu.make_async_copy(src.at[pl.ds(r * rp, rp), pl.ds(c * 128, 128)],
                                      dst.at[c, pl.ds(r * rp, rp), :],
                                      sem).start(priority=n % 2)
                n += 1

    pltpu.make_async_copy(x_hbm, x_s, wsem).start()
    pltpu.make_async_copy(wr_hbm, wr_s, wsem).start()
    start_w(wq_hbm, wq_b, wsem, 320)
    start_w(wo_hbm, wo_b, wsem, 96)
    start_w(wg_hbm, wg_b, wsem, 320)
    start_w(wu_hbm, wu_b, wsem, 320)
    start_w(wd_hbm, wd_b, wsem, 96)
    start_k(0)
    start_v(0)
    start_k(1)
    start_v(1)
    start_k(2)

    for buf in (x_s, wr_s, wq_b, wo_b, wg_b, wu_b, wd_b):
        wait_all(buf, wsem)
    x_all = x_s[...].astype(f32)
    wr = wr_s[...].astype(f32)
    wr_row = jnp.concatenate([wr[i:i + 1, :] for i in range(ND)], axis=1)

    row = jax.lax.broadcasted_iota(jnp.int32, (HG, GW), 0)
    col = jax.lax.broadcasted_iota(jnp.int32, (HG, GW), 1)
    mask = (col >= row * DH) & (col < row * DH + DH)
    row4 = jax.lax.broadcasted_iota(jnp.int32, (B, D), 0)

    def wo_proj(t, r0, nr):
        return jnp.concatenate(
            [_mm(t, _as_bf16(wo32[n, pl.ds(r0, nr), :])) for n in range(ND)], axis=1)

    def attention1(x, b):
        h = _ln(x).astype(bf16)

        def group(g, acc):
            j = b * NG + g
            q = jnp.concatenate(
                [_mm(h, _as_bf16(wq32[g * NT + t])) for t in range(NT)], axis=1)
            qbd = jnp.where(mask, q, 0.0).astype(bf16)
            wait_all(kbuf.at[j], ksem.at[g])

            @pl.when(g == 3)
            def _():
                start_k(j + 1)
            s = jnp.concatenate(
                [_mm(qbd, _as_bf16(k32[j, c].reshape(HG * DH2, 128))) for c in range(NC)],
                axis=1) * SCALE
            m = jnp.max(s, axis=-1, keepdims=True)
            p = jnp.exp(s - m)
            l = jnp.sum(p, axis=-1, keepdims=True)
            pb = p.astype(bf16)
            rl = 1.0 / l
            for part in range(HG // VP):
                wait_all(vbuf.at[j, :, pl.ds(part * VP, VP)], vsem.at[(g % 2) * (HG // VP) + part])
                if part == HG // VP - 1:
                    @pl.when(g == 3)
                    def _():
                        start_v(j + 1)
                o = None
                for c in range(NC):
                    d = jax.lax.dot_general(
                        pb[:, 128 * c:128 * (c + 1)],
                        _as_bf16(v32[j, c, pl.ds(part * VP, VP)].reshape(VP * DH2, 128)),
                        (((1,), (1,)), ((), ())), preferred_element_type=f32)
                    o = d if o is None else o + d
                cols = slice(part * VP * DH, (part + 1) * VP * DH)
                om = jnp.where(mask[:, cols], o * rl, 0.0).astype(bf16)
                acc = acc + wo_proj(om, pl.multiple_of(g * (GW // 2) + part * VP * DH2, 8), VP * DH2)

            @pl.when((g == 0) | (g == 2))
            def _():
                start_v(j + 2 - g // 2)

            @pl.when(g == 1)
            def _():
                start_k(j + 2)
            return acc

        acc = jax.lax.fori_loop(0, NG, group, jnp.zeros((HG, D), f32))
        return x + jnp.broadcast_to(jnp.sum(acc, axis=0, keepdims=True), (HG, D))

    lane = jax.lax.broadcasted_iota(jnp.int32, (HG, 128), 1)
    sub = jax.lax.broadcasted_iota(jnp.int32, (HG, 128), 0)
    dl = lane - 2 * sub

    def spread(v, rblk):
        t, base = divmod(16 * rblk, 128)
        vt = v[:, 128 * t:128 * (t + 1)]
        even = jnp.sum(jnp.where(dl == base, vt, 0.0), axis=-1, keepdims=True)
        odd = jnp.sum(jnp.where(dl == base + 1, vt, 0.0), axis=-1, keepdims=True)
        return even, odd

    def rowsum(a):
        return jnp.broadcast_to(jnp.sum(a, axis=0, keepdims=True), a.shape)

    def attention2(x, b, feed):
        h = _ln(x).astype(bf16)
        st = {'acc': None}
        N = NG * NT

        def tile_mask(t):
            c = lane + 128 * t
            return (c >= sub * DH) & (c < sub * DH + DH)

        def vpu_q():
            hr = h.astype(f32)
            acc = {}
            for rb in range(D // 16):
                even, odd = spread(hr, rb)
                if 'gate' in st:
                    even = even + st['gate']
                for u in range(N - VQ, N):
                    w = wq32[u, pl.ds(8 * rb, 8), :]
                    d = _lo(w) * even + _hi(w) * odd
                    acc[u] = d if rb == 0 else acc[u] + d
                yield
            for u in range(N - VQ, N):
                st['q', u] = jnp.where(tile_mask(u % UT), rowsum(acc[u]), 0.0).astype(bf16)

        vq = vpu_q()

        def q_tile(u):
            if u >= N - VQ:
                return
            for _ in range(VQP):
                next(vq, None)
            q = _mm(h, _as_bf16(wq32[u]))
            st['gate'] = q * 0.0
            st['q', u] = jnp.where(tile_mask(u % UT), q, 0.0).astype(bf16)

        def k_rows(c, u):
            hd, r0 = divmod(64 * u, DH2)
            g, h0 = divmod(hd, HG)
            j = b * NG + g
            if r0 + 64 <= DH2:
                return k32[j, c, h0, pl.ds(r0, 64), :]
            return jnp.concatenate([k32[j, c, h0, pl.ds(r0, DH2 - r0), :],
                                    k32[j, c, h0 + 1, pl.ds(0, 64 - (DH2 - r0)), :]], axis=0)

        def s_tile(u):
            k, t = divmod(u, UT)
            qt = st.pop(('q', u))
            d = jnp.concatenate([_mm(qt, _as_bf16(k_rows(c, u))) for c in range(NC)], axis=1)
            st['s', k] = d if t == 0 else st['s', k] + d
            if t == UT - 1:
                sa = st.pop(('s', k))
                m = jnp.max(sa, axis=-1, keepdims=True)
                p = jnp.exp2((sa - m) * (SCALE * LOG2E))
                st['p', k] = p
                st['rl', k] = 1.0 / jnp.sum(p, axis=-1, keepdims=True)

        def fac(hd):
            if ('f', hd) not in st:
                st['f', hd] = jnp.broadcast_to(st['rl', hd // U][hd % U:hd % U + 1, :], (HG, 128))
            return st['f', hd]

        def v_tile(u):
            p = st['p', u // UT]
            tile = jnp.zeros((HG, 128), f32)
            for c in range(128 * u, 128 * u + 128, 16):
                hd, r = c // DH, (c % DH) // 16
                g, hh = divmod(hd, HG)
                if ('pb', hd) not in st:
                    hu = hd % U
                    st['pb', hd] = [jnp.broadcast_to(p[hu:hu + 1, 128 * i:128 * (i + 1)], (HG, 128))
                                    for i in range(NC)]
                pb = st['pb', hd]
                acc = []
                for half in range(2):
                    alo = ahi = None
                    for i in range(4 * half, 4 * half + 4):
                        w = v32[b * NG + g, i, hh, pl.ds(8 * r, 8), :]
                        lo = _lo(w) * pb[i]
                        hi = _hi(w) * pb[i]
                        alo = lo if alo is None else alo + lo
                        ahi = hi if ahi is None else ahi + hi
                    acc.append((alo, ahi))
                rlo = jnp.sum(acc[0][0], axis=-1, keepdims=True) + jnp.sum(acc[1][0], axis=-1, keepdims=True)
                rhi = jnp.sum(acc[0][1], axis=-1, keepdims=True) + jnp.sum(acc[1][1], axis=-1, keepdims=True)
                if u >= VWO:
                    rlo = (rlo * fac(hd)).astype(bf16).astype(f32)
                    rhi = (rhi * fac(hd)).astype(bf16).astype(f32)
                    for n in range(ND):
                        w = wo32[n, pl.ds(c // 2, 8), :]
                        d = _lo(w) * rlo + _hi(w) * rhi
                        st['vacc', n] = st['vacc', n] + d if ('vacc', n) in st else d
                else:
                    base = c % 128
                    tile = jnp.where(dl == base, rlo, jnp.where(dl == base + 1, rhi, tile))
            if u < VWO:
                ha, hb = (128 * u) // DH, (128 * u + 127) // DH
                f = fac(ha) if ha == hb else jnp.where(lane < hb * DH - 128 * u, fac(ha), fac(hb))
                st['t', u] = (tile * f).astype(bf16)

        def w_tile(u):
            if u >= VWO:
                return
            d = wo_proj(st.pop(('t', u)), 64 * u, 64)
            st['acc'] = d if st['acc'] is None else st['acc'] + d

        SL = SLEAD * UT
        for m in range(-SL - QLEAD, N + WLAG):
            if m == MFEED:
                feed()
            if 0 <= m + SL + QLEAD < N:
                q_tile(m + SL + QLEAD)
            if 0 <= m + SL < N:
                s_tile(m + SL)
            if 0 <= m < N:
                v_tile(m)
            if 0 <= m - WLAG < N:
                w_tile(m - WLAG)
        for _ in vq:
            pass
        acc = st['acc'] + jnp.concatenate([st['vacc', n] for n in range(ND)], axis=1)
        return x + jnp.broadcast_to(jnp.sum(acc, axis=0, keepdims=True), (HG, D))

    def ffn(x):
        h = _ln(x)
        r = jnp.sum(h * wr_row, axis=-1, keepdims=True)
        hb = h.astype(bf16)
        a = [None] * NF
        accs = {}
        gate = [None]

        def act(g, u):
            return (g * jax.nn.sigmoid(g) * u).astype(bf16)

        def vpu_blocks():
            hr = hb.astype(f32)
            for rb in range(D // 16):
                even, odd = spread(hr, rb)
                if gate[0] is not None:
                    even = even + gate[0]
                for t in range(NF - NV, NF):
                    for nm, w32 in (('g', wg32), ('u', wu32)):
                        w = w32[t, pl.ds(8 * rb, 8), :]
                        d = _lo(w) * even + _hi(w) * odd
                        accs[nm, t] = d if rb == 0 else accs[nm, t] + d
                yield

        blocks = vpu_blocks()
        per = -(-(D // 16) // (NF - NV))
        for t in range(NF - NV):
            for _ in range(per):
                next(blocks, None)
            g = _mm(hb, _as_bf16(wg32[t]))
            u = _mm(hb, _as_bf16(wu32[t]))
            gate[0] = g * 0.0
            a[t] = act(g, u)
        for _ in blocks:
            pass
        for t in range(NF - NV, NF):
            a[t] = act(rowsum(accs['g', t]), rowsum(accs['u', t]))
        nk = NF - DV
        am = jnp.concatenate(a[:nk], axis=1)
        y = [_mm(am, _as_bf16(wd32[n, pl.ds(0, 64 * nk), :])) for n in range(ND)]
        yv = [None] * ND
        for t in range(nk, NF):
            af = a[t].astype(f32)
            for rb in range(8):
                even, odd = spread(af, rb)
                for n in range(ND):
                    w = wd32[n, pl.ds(64 * t + 8 * rb, 8), :]
                    d = _lo(w) * even + _hi(w) * odd
                    yv[n] = d if yv[n] is None else yv[n] + d
        y = jnp.concatenate([y[n] + rowsum(yv[n]) for n in range(ND)], axis=1)
        return x + h + y * jax.nn.sigmoid(r)

    def batch(b, out):
        xb = jnp.sum(jnp.where(row4 == b, x_all, 0.0), axis=0, keepdims=True)
        x = jnp.broadcast_to(xb, (HG, D))
        x = attention1(x, b)
        x = ffn(x)
        start_k(b * NG + 5)
        x = attention2(x, b, lambda: start_v(b * NG + 5))
        start_k(b * NG + 6)
        x = ffn(x)
        return jnp.where(row4 == b, x[:B, :], out)

    out = jax.lax.fori_loop(0, B - 1, batch, jnp.zeros((B, D), f32))
    out = batch(B - 1, out)
    o_ref[...] = out.astype(o_ref.dtype)


@jax.jit
def pallas_interleave_layers__sliding_block_cached__moe_arch_mod__decode_kernel(
    A_x: jax.Array,
    A_k_cache: jax.Array,
    A_v_cache: jax.Array,
    A_wq: jax.Array,
    A_wo: jax.Array,
    B_x: jax.Array,
    B_w_r: jax.Array,
    B_w_gate: jax.Array,
    B_w_up: jax.Array,
    B_w_down: jax.Array,
):
    del B_x
    k_t = jnp.transpose(A_k_cache, (0, 1, 3, 2))
    v_t = jnp.transpose(A_v_cache, (0, 1, 3, 2))
    any_spec = pl.BlockSpec(memory_space=pl.ANY)
    out = pl.pallas_call(
        _kernel,
        out_shape=jax.ShapeDtypeStruct((B, D), A_x.dtype),
        in_specs=[any_spec] * 9,
        out_specs=pl.BlockSpec(memory_space=pltpu.VMEM),
        scratch_shapes=[
            pltpu.VMEM((NJ, NC, HG, DH, 128), bf16),
            pltpu.VMEM((NJ, NC, HG, DH, 128), bf16),
            pltpu.VMEM((H * DH // 128, D, 128), bf16),
            pltpu.VMEM((ND, H * DH, 128), bf16),
            pltpu.VMEM((NF, D, 128), bf16),
            pltpu.VMEM((NF, D, 128), bf16),
            pltpu.VMEM((ND, F, 128), bf16),
            pltpu.VMEM((B, D), bf16),
            pltpu.VMEM((ND, 128), bf16),
            pltpu.SemaphoreType.DMA((NG,)),
            pltpu.SemaphoreType.DMA((2 * HG // VP,)),
            pltpu.SemaphoreType.DMA(()),
        ],
        compiler_params=pltpu.CompilerParams(vmem_limit_bytes=126 * 1024 * 1024),
    )(A_x.reshape(B, D), B_w_r.reshape(ND, 128), k_t, v_t,
      A_wq, A_wo, B_w_gate, B_w_up, B_w_down)
    return out.reshape(B, 1, D)
```

```python
import jax
import jax.numpy as jnp
from jax.experimental import pallas as pl
from jax.experimental.pallas import tpu as pltpu

B, D, H, DH, SK, F = 4, 640, 32, 192, 4096, 1536
W = min(4096, max(256, SK // 4))
HG = 8
NG = H // HG
NJ = B * NG
GW = HG * DH
DH2 = DH // 2
NC = W // 128
NT = GW // 128
ND = D // 128
NF = F // 128
EPS = 1e-5
SCALE = DH ** -0.5
LOG2E = 1.4426950408889634
VP = 2
U = 4
UT = U * DH // 128
SLEAD = 3
QLEAD = 2
WLAG = 24
MFEED = 16
VQ, VQP = 4, 5
VWO = 46
NV, DV = 2, 4

f32, bf16, u32 = jnp.float32, jnp.bfloat16, jnp.uint32


def _ln(x):
    m = jnp.mean(x, axis=-1, keepdims=True)
    m2 = jnp.mean(x * x, axis=-1, keepdims=True)
    v = jnp.maximum(m2 - m * m, 0.0)
    return (x - m) * jax.lax.rsqrt(v + EPS)


def _as_bf16(w):
    return pltpu.bitcast(w, bf16)


def _lo(w):
    return pltpu.bitcast(w << 16, f32)


def _hi(w):
    return pltpu.bitcast(w & jnp.uint32(0xFFFF0000), f32)


def _mm(a, w):
    return jnp.dot(a, w, preferred_element_type=f32)


def _kernel(x_hbm, wr_hbm, k_hbm, v_hbm, wq_hbm, wo_hbm, wg_hbm, wu_hbm, wd_hbm,
            o_ref,
            kbuf, vbuf, wq_b, wo_b, wg_b, wu_b, wd_b, x_s, wr_s,
            ksem, vsem, wsem):
    k32, v32 = kbuf.bitcast(u32), vbuf.bitcast(u32)
    wq32, wo32 = wq_b.bitcast(u32), wo_b.bitcast(u32)
    wg32, wu32, wd32 = wg_b.bitcast(u32), wu_b.bitcast(u32), wd_b.bitcast(u32)

    def start_kv(src, dst, sems, j, hp, sem_heads, ring):
        b = j // NG
        g = j % NG

        def heads(i, carry):
            sem = sems.at[(j % ring) * (HG // sem_heads) + (i * hp) // sem_heads]
            for c in range(NC):
                pltpu.make_async_copy(
                    src.at[b, pl.ds(g * HG + i * hp, hp), :, pl.ds(SK - W + c * 128, 128)],
                    dst.at[j, c, pl.ds(i * hp, hp)],
                    sem).start(priority=c % 2)
            return carry

        jax.lax.fori_loop(0, HG // hp, heads, 0)

    def start_k(j, hp=1):
        if isinstance(j, int):
            if j < NJ:
                start_kv(k_hbm, kbuf, ksem, j, hp, HG, NG)
            return

        @pl.when(j < NJ)
        def _():
            start_kv(k_hbm, kbuf, ksem, j, hp, HG, NG)

    def start_v(j, hp=1):
        if isinstance(j, int):
            if j < NJ:
                start_kv(v_hbm, vbuf, vsem, j, hp, VP, 2)
            return

        @pl.when(j < NJ)
        def _():
            start_kv(v_hbm, vbuf, vsem, j, hp, VP, 2)

    def wait_all(buf, sem):
        pltpu.make_async_copy(buf, buf, sem).wait()

    def start_w(src, dst, sem, rp):
        rows, cols = src.shape
        n = 0
        for r in range(rows // rp):
            for c in range(cols // 128):
                pltpu.make_async_copy(src.at[pl.ds(r * rp, rp), pl.ds(c * 128, 128)],
                                      dst.at[c, pl.ds(r * rp, rp), :],
                                      sem).start(priority=n % 2)
                n += 1

    pltpu.make_async_copy(x_hbm, x_s, wsem).start()
    pltpu.make_async_copy(wr_hbm, wr_s, wsem).start()
    start_w(wq_hbm, wq_b, wsem, 320)
    start_w(wo_hbm, wo_b, wsem, 96)
    start_w(wg_hbm, wg_b, wsem, 320)
    start_w(wu_hbm, wu_b, wsem, 320)
    start_w(wd_hbm, wd_b, wsem, 96)
    start_k(0)
    start_v(0)
    start_k(1)
    start_v(1)
    start_k(2)

    for buf in (x_s, wr_s, wq_b, wo_b, wg_b, wu_b, wd_b):
        wait_all(buf, wsem)
    x_all = x_s[...].astype(f32)
    wr = wr_s[...].astype(f32)
    wr_row = jnp.concatenate([wr[i:i + 1, :] for i in range(ND)], axis=1)

    row = jax.lax.broadcasted_iota(jnp.int32, (HG, GW), 0)
    col = jax.lax.broadcasted_iota(jnp.int32, (HG, GW), 1)
    mask = (col >= row * DH) & (col < row * DH + DH)
    row4 = jax.lax.broadcasted_iota(jnp.int32, (B, D), 0)

    def wo_proj(t, r0, nr):
        return jnp.concatenate(
            [_mm(t, _as_bf16(wo32[n, pl.ds(r0, nr), :])) for n in range(ND)], axis=1)

    lane = jax.lax.broadcasted_iota(jnp.int32, (HG, 128), 1)
    sub = jax.lax.broadcasted_iota(jnp.int32, (HG, 128), 0)
    dl = lane - 2 * sub

    def row_bcast(p, r):
        return [jnp.broadcast_to(p[r:r + 1, 128 * i:128 * (i + 1)], (HG, 128)) for i in range(NC)]

    def pv_block(j, hh, r, pb):
        acc = []
        for half in range(2):
            alo = ahi = None
            for i in range(4 * half, 4 * half + 4):
                w = v32[j, i, hh, pl.ds(8 * r, 8), :]
                lo = _lo(w) * pb[i]
                hi = _hi(w) * pb[i]
                alo = lo if alo is None else alo + lo
                ahi = hi if ahi is None else ahi + hi
            acc.append((alo, ahi))
        rlo = jnp.sum(acc[0][0], axis=-1, keepdims=True) + jnp.sum(acc[1][0], axis=-1, keepdims=True)
        rhi = jnp.sum(acc[0][1], axis=-1, keepdims=True) + jnp.sum(acc[1][1], axis=-1, keepdims=True)
        return rlo, rhi

    def when(cond):
        if isinstance(cond, bool):
            return (lambda f: f()) if cond else (lambda f: None)
        return pl.when(cond)

    def attention1(x, b):
        h = _ln(x).astype(bf16)

        def aligned(i):
            return i if isinstance(i, int) else pl.multiple_of(i, 8)

        def last_part(j, g, p, pb, rl):
            t0 = NT - 3
            out = None
            for t in (t0 + 1, t0, t0 + 2):
                if t == t0 + 1:
                    o = None
                    for c in range(NC):
                        vrows = jnp.concatenate([v32[j, c, HG - 2, pl.ds(64, 32), :],
                                                 v32[j, c, HG - 1, pl.ds(0, 32), :]], axis=0)
                        d = jax.lax.dot_general(pb[:, 128 * c:128 * (c + 1)], _as_bf16(vrows),
                                                (((1,), (1,)), ((), ())), preferred_element_type=f32)
                        o = d if o is None else o + d
                    tile = jnp.where(mask[:, 128 * t:128 * (t + 1)], o * rl, 0.0)
                else:
                    hh = (128 * t) // DH
                    pbs = row_bcast(p, hh)
                    tile = jnp.zeros((HG, 128), f32)
                    for c in range(128 * t, 128 * t + 128, 16):
                        rlo, rhi = pv_block(j, hh, (c % DH) // 16, pbs)
                        tile = jnp.where(dl == c % 128, rlo, jnp.where(dl == c % 128 + 1, rhi, tile))
                    tile = tile * jnp.broadcast_to(rl[hh:hh + 1, :], (HG, 128))
                d = wo_proj(tile.astype(bf16), g * (GW // 2) + 64 * t, 64)
                out = d if out is None else out + d
            return out

        def group(g, acc):
            j = b * NG + g
            q = jnp.concatenate(
                [_mm(h, _as_bf16(wq32[g * NT + t])) for t in range(NT)], axis=1)
            qbd = jnp.where(mask, q, 0.0).astype(bf16)
            wait_all(kbuf.at[j], ksem.at[g])

            @when(g == 3)
            def _():
                start_k(j + 1)
            s = jnp.concatenate(
                [_mm(qbd, _as_bf16(k32[j, c].reshape(HG * DH2, 128))) for c in range(NC)],
                axis=1) * SCALE
            m = jnp.max(s, axis=-1, keepdims=True)
            p = jnp.exp(s - m)
            l = jnp.sum(p, axis=-1, keepdims=True)
            pb = p.astype(bf16)
            rl = 1.0 / l
            for part in range(HG // VP):
                wait_all(vbuf.at[j, :, pl.ds(part * VP, VP)], vsem.at[(g % 2) * (HG // VP) + part])
                if part == HG // VP - 1:
                    @when(g == 3)
                    def _():
                        start_v(j + 1)
                if isinstance(g, int) and part == HG // VP - 1:
                    acc = acc + last_part(j, g, p, pb, rl)
                    break
                o = None
                for c in range(NC):
                    d = jax.lax.dot_general(
                        pb[:, 128 * c:128 * (c + 1)],
                        _as_bf16(v32[j, c, pl.ds(part * VP, VP)].reshape(VP * DH2, 128)),
                        (((1,), (1,)), ((), ())), preferred_element_type=f32)
                    o = d if o is None else o + d
                cols = slice(part * VP * DH, (part + 1) * VP * DH)
                om = jnp.where(mask[:, cols], o * rl, 0.0).astype(bf16)
                acc = acc + wo_proj(om, aligned(g * (GW // 2) + part * VP * DH2), VP * DH2)

            @when((g % 2) == 0)
            def _():
                start_v(j + 2 - g // 2)

            @when(g == 1)
            def _():
                start_k(j + 2)
            return acc

        acc = jnp.zeros((HG, D), f32)
        if isinstance(b, int):
            acc = group(NG - 1, jax.lax.fori_loop(0, NG - 1, group, acc))
        else:
            acc = jax.lax.fori_loop(0, NG, group, acc)
        return x + jnp.broadcast_to(jnp.sum(acc, axis=0, keepdims=True), (HG, D))

    def spread(v, rblk):
        t, base = divmod(16 * rblk, 128)
        vt = v[:, 128 * t:128 * (t + 1)]
        even = jnp.sum(jnp.where(dl == base, vt, 0.0), axis=-1, keepdims=True)
        odd = jnp.sum(jnp.where(dl == base + 1, vt, 0.0), axis=-1, keepdims=True)
        return even, odd

    def rowsum(a):
        return jnp.broadcast_to(jnp.sum(a, axis=0, keepdims=True), a.shape)

    def attention2(x, b, feed):
        h = _ln(x).astype(bf16)
        st = {'acc': None}
        N = NG * NT

        def tile_mask(t):
            c = lane + 128 * t
            return (c >= sub * DH) & (c < sub * DH + DH)

        def vpu_q():
            hr = h.astype(f32)
            acc = {}
            for rb in range(D // 16):
                even, odd = spread(hr, rb)
                if 'gate' in st:
                    even = even + st['gate']
                for u in range(N - VQ, N):
                    w = wq32[u, pl.ds(8 * rb, 8), :]
                    d = _lo(w) * even + _hi(w) * odd
                    acc[u] = d if rb == 0 else acc[u] + d
                yield
            for u in range(N - VQ, N):
                st['q', u] = jnp.where(tile_mask(u % UT), rowsum(acc[u]), 0.0).astype(bf16)

        vq = vpu_q()

        def q_tile(u):
            if u >= N - VQ:
                return
            for _ in range(VQP):
                next(vq, None)
            q = _mm(h, _as_bf16(wq32[u]))
            st['gate'] = q * 0.0
            st['q', u] = jnp.where(tile_mask(u % UT), q, 0.0).astype(bf16)

        def k_rows(c, u):
            hd, r0 = divmod(64 * u, DH2)
            g, h0 = divmod(hd, HG)
            j = b * NG + g
            if r0 + 64 <= DH2:
                return k32[j, c, h0, pl.ds(r0, 64), :]
            return jnp.concatenate([k32[j, c, h0, pl.ds(r0, DH2 - r0), :],
                                    k32[j, c, h0 + 1, pl.ds(0, 64 - (DH2 - r0)), :]], axis=0)

        def s_tile(u):
            k, t = divmod(u, UT)
            qt = st.pop(('q', u))
            d = jnp.concatenate([_mm(qt, _as_bf16(k_rows(c, u))) for c in range(NC)], axis=1)
            st['s', k] = d if t == 0 else st['s', k] + d
            if t == UT - 1:
                sa = st.pop(('s', k))
                m = jnp.max(sa, axis=-1, keepdims=True)
                p = jnp.exp2((sa - m) * (SCALE * LOG2E))
                st['p', k] = p
                st['rl', k] = 1.0 / jnp.sum(p, axis=-1, keepdims=True)

        def fac(hd):
            if ('f', hd) not in st:
                st['f', hd] = jnp.broadcast_to(st['rl', hd // U][hd % U:hd % U + 1, :], (HG, 128))
            return st['f', hd]

        def v_tile(u):
            p = st['p', u // UT]
            tile = jnp.zeros((HG, 128), f32)
            for c in range(128 * u, 128 * u + 128, 16):
                hd, r = c // DH, (c % DH) // 16
                g, hh = divmod(hd, HG)
                if ('pb', hd) not in st:
                    st['pb', hd] = row_bcast(p, hd % U)
                rlo, rhi = pv_block(b * NG + g, hh, r, st['pb', hd])
                if u >= VWO:
                    rlo = (rlo * fac(hd)).astype(bf16).astype(f32)
                    rhi = (rhi * fac(hd)).astype(bf16).astype(f32)
                    for n in range(ND):
                        w = wo32[n, pl.ds(c // 2, 8), :]
                        d = _lo(w) * rlo + _hi(w) * rhi
                        st['vacc', n] = st['vacc', n] + d if ('vacc', n) in st else d
                else:
                    base = c % 128
                    tile = jnp.where(dl == base, rlo, jnp.where(dl == base + 1, rhi, tile))
            if u < VWO:
                ha, hb = (128 * u) // DH, (128 * u + 127) // DH
                f = fac(ha) if ha == hb else jnp.where(lane < hb * DH - 128 * u, fac(ha), fac(hb))
                st['t', u] = (tile * f).astype(bf16)

        def w_tile(u):
            if u >= VWO:
                return
            d = wo_proj(st.pop(('t', u)), 64 * u, 64)
            st['acc'] = d if st['acc'] is None else st['acc'] + d

        SL = SLEAD * UT
        for m in range(-SL - QLEAD, N + WLAG):
            if m == MFEED:
                feed()
            if 0 <= m + SL + QLEAD < N:
                q_tile(m + SL + QLEAD)
            if 0 <= m + SL < N:
                s_tile(m + SL)
            if 0 <= m < N:
                v_tile(m)
            if 0 <= m - WLAG < N:
                w_tile(m - WLAG)
        for _ in vq:
            pass
        acc = st['acc'] + jnp.concatenate([st['vacc', n] for n in range(ND)], axis=1)
        return x + jnp.broadcast_to(jnp.sum(acc, axis=0, keepdims=True), (HG, D))

    def ffn(x):
        h = _ln(x)
        r = jnp.sum(h * wr_row, axis=-1, keepdims=True)
        hb = h.astype(bf16)
        a = [None] * NF
        accs = {}
        gate = [None]

        def act(g, u):
            return (g * jax.nn.sigmoid(g) * u).astype(bf16)

        def vpu_blocks():
            hr = hb.astype(f32)
            for rb in range(D // 16):
                even, odd = spread(hr, rb)
                if gate[0] is not None:
                    even = even + gate[0]
                for t in range(NF - NV, NF):
                    for nm, w32 in (('g', wg32), ('u', wu32)):
                        w = w32[t, pl.ds(8 * rb, 8), :]
                        d = _lo(w) * even + _hi(w) * odd
                        accs[nm, t] = d if rb == 0 else accs[nm, t] + d
                yield

        blocks = vpu_blocks()
        per = -(-(D // 16) // (NF - NV))
        for t in range(NF - NV):
            for _ in range(per):
                next(blocks, None)
            g = _mm(hb, _as_bf16(wg32[t]))
            u = _mm(hb, _as_bf16(wu32[t]))
            gate[0] = g * 0.0
            a[t] = act(g, u)
        for _ in blocks:
            pass
        for t in range(NF - NV, NF):
            a[t] = act(rowsum(accs['g', t]), rowsum(accs['u', t]))
        nk = NF - DV
        am = jnp.concatenate(a[:nk], axis=1)
        y = [_mm(am, _as_bf16(wd32[n, pl.ds(0, 64 * nk), :])) for n in range(ND)]
        yv = [None] * ND
        for t in range(nk, NF):
            af = a[t].astype(f32)
            for rb in range(8):
                even, odd = spread(af, rb)
                for n in range(ND):
                    w = wd32[n, pl.ds(64 * t + 8 * rb, 8), :]
                    d = _lo(w) * even + _hi(w) * odd
                    yv[n] = d if yv[n] is None else yv[n] + d
        y = jnp.concatenate([y[n] + rowsum(yv[n]) for n in range(ND)], axis=1)
        return x + h + y * jax.nn.sigmoid(r)

    def batch(b, out):
        xb = jnp.sum(jnp.where(row4 == b, x_all, 0.0), axis=0, keepdims=True)
        x = jnp.broadcast_to(xb, (HG, D))
        x = attention1(x, b)
        x = ffn(x)
        start_k(b * NG + 5)
        x = attention2(x, b, lambda: start_v(b * NG + 5))
        start_k(b * NG + 6)
        x = ffn(x)
        return jnp.where(row4 == b, x[:B, :], out)

    out = jax.lax.fori_loop(0, B - 1, batch, jnp.zeros((B, D), f32))
    out = batch(B - 1, out)
    o_ref[...] = out.astype(o_ref.dtype)


@jax.jit
def pallas_interleave_layers__sliding_block_cached__moe_arch_mod__decode_kernel(
    A_x: jax.Array,
    A_k_cache: jax.Array,
    A_v_cache: jax.Array,
    A_wq: jax.Array,
    A_wo: jax.Array,
    B_x: jax.Array,
    B_w_r: jax.Array,
    B_w_gate: jax.Array,
    B_w_up: jax.Array,
    B_w_down: jax.Array,
):
    del B_x
    k_t = jnp.transpose(A_k_cache, (0, 1, 3, 2))
    v_t = jnp.transpose(A_v_cache, (0, 1, 3, 2))
    any_spec = pl.BlockSpec(memory_space=pl.ANY)
    out = pl.pallas_call(
        _kernel,
        out_shape=jax.ShapeDtypeStruct((B, D), A_x.dtype),
        in_specs=[any_spec] * 9,
        out_specs=pl.BlockSpec(memory_space=pltpu.VMEM),
        scratch_shapes=[
            pltpu.VMEM((NJ, NC, HG, DH, 128), bf16),
            pltpu.VMEM((NJ, NC, HG, DH, 128), bf16),
            pltpu.VMEM((H * DH // 128, D, 128), bf16),
            pltpu.VMEM((ND, H * DH, 128), bf16),
            pltpu.VMEM((NF, D, 128), bf16),
            pltpu.VMEM((NF, D, 128), bf16),
            pltpu.VMEM((ND, F, 128), bf16),
            pltpu.VMEM((B, D), bf16),
            pltpu.VMEM((ND, 128), bf16),
            pltpu.SemaphoreType.DMA((NG,)),
            pltpu.SemaphoreType.DMA((2 * HG // VP,)),
            pltpu.SemaphoreType.DMA(()),
        ],
        compiler_params=pltpu.CompilerParams(vmem_limit_bytes=126 * 1024 * 1024),
    )(A_x.reshape(B, D), B_w_r.reshape(ND, 128), k_t, v_t,
      A_wq, A_wo, B_w_gate, B_w_up, B_w_down)
    return out.reshape(B, 1, D)
```

```python
import jax
import jax.numpy as jnp
from jax.experimental import pallas as pl
from jax.experimental.pallas import tpu as pltpu

B, D, H, DH, SK, F = 4, 640, 32, 192, 4096, 1536
W = min(4096, max(256, SK // 4))
HG = 8
NG = H // HG
NJ = B * NG
GW = HG * DH
DH2 = DH // 2
NC = W // 128
NT = GW // 128
ND = D // 128
NF = F // 128
EPS = 1e-5
SCALE = DH ** -0.5
LOG2E = 1.4426950408889634
VP = 2
U = 4
UT = U * DH // 128
SLEAD = 3
QLEAD = 2
WLAG = 24
MFEED = 16
VQ, VQP = 4, 5
VWO = 46
NV, DV = 2, 4

f32, bf16, u32 = jnp.float32, jnp.bfloat16, jnp.uint32


def _ln(x):
    m = jnp.mean(x, axis=-1, keepdims=True)
    m2 = jnp.mean(x * x, axis=-1, keepdims=True)
    v = jnp.maximum(m2 - m * m, 0.0)
    return (x - m) * jax.lax.rsqrt(v + EPS)


def _as_bf16(w):
    return pltpu.bitcast(w, bf16)


def _lo(w):
    return pltpu.bitcast(w << 16, f32)


def _hi(w):
    return pltpu.bitcast(w & jnp.uint32(0xFFFF0000), f32)


def _mm(a, w):
    return jnp.dot(a, w, preferred_element_type=f32)


def _kernel(x_hbm, wr_hbm, k_hbm, v_hbm, wq_hbm, wo_hbm, wg_hbm, wu_hbm, wd_hbm,
            o_ref,
            kbuf, vbuf, wq_b, wo_b, wg_b, wu_b, wd_b, x_s, wr_s,
            ksem, vsem, wsem):
    k32, v32 = kbuf.bitcast(u32), vbuf.bitcast(u32)
    wq32, wo32 = wq_b.bitcast(u32), wo_b.bitcast(u32)
    wg32, wu32, wd32 = wg_b.bitcast(u32), wu_b.bitcast(u32), wd_b.bitcast(u32)

    def start_kv(src, dst, sems, j, sem_heads, ring):
        b = j // NG
        g = j % NG

        def head(i, carry):
            sem = sems.at[(j % ring) * (HG // sem_heads) + i // sem_heads]
            for c in range(NC):
                pltpu.make_async_copy(
                    src.at[b, g * HG + i, :, pl.ds(SK - W + c * 128, 128)],
                    dst.at[j, c, i],
                    sem).start(priority=c % 2)
            return carry

        jax.lax.fori_loop(0, HG, head, 0)

    def when(cond):
        if isinstance(cond, bool):
            return (lambda f: f()) if cond else (lambda f: None)
        return pl.when(cond)

    def start_k(j):
        @when(j < NJ)
        def _():
            start_kv(k_hbm, kbuf, ksem, j, HG, NG)

    def start_v(j):
        @when(j < NJ)
        def _():
            start_kv(v_hbm, vbuf, vsem, j, VP, 2)

    def wait_all(buf, sem):
        pltpu.make_async_copy(buf, buf, sem).wait()

    def start_w(src, dst, sem, rp):
        rows, cols = src.shape
        n = 0
        for r in range(rows // rp):
            for c in range(cols // 128):
                pltpu.make_async_copy(src.at[pl.ds(r * rp, rp), pl.ds(c * 128, 128)],
                                      dst.at[c, pl.ds(r * rp, rp), :],
                                      sem).start(priority=n % 2)
                n += 1

    pltpu.make_async_copy(x_hbm, x_s, wsem).start()
    pltpu.make_async_copy(wr_hbm, wr_s, wsem).start()
    start_w(wq_hbm, wq_b, wsem, 320)
    start_w(wo_hbm, wo_b, wsem, 96)
    start_w(wg_hbm, wg_b, wsem, 320)
    start_w(wu_hbm, wu_b, wsem, 320)
    start_w(wd_hbm, wd_b, wsem, 96)
    start_k(0)
    start_v(0)
    start_k(1)
    start_v(1)
    start_k(2)

    for buf in (x_s, wr_s, wq_b, wo_b, wg_b, wu_b, wd_b):
        wait_all(buf, wsem)
    x_all = x_s[...].astype(f32)
    wr = wr_s[...].astype(f32)
    wr_row = jnp.concatenate([wr[i:i + 1, :] for i in range(ND)], axis=1)

    row = jax.lax.broadcasted_iota(jnp.int32, (HG, GW), 0)
    col = jax.lax.broadcasted_iota(jnp.int32, (HG, GW), 1)
    mask = (col >= row * DH) & (col < row * DH + DH)
    row4 = jax.lax.broadcasted_iota(jnp.int32, (B, D), 0)

    def wo_proj(t, r0, nr):
        return jnp.concatenate(
            [_mm(t, _as_bf16(wo32[n, pl.ds(r0, nr), :])) for n in range(ND)], axis=1)

    lane = jax.lax.broadcasted_iota(jnp.int32, (HG, 128), 1)
    sub = jax.lax.broadcasted_iota(jnp.int32, (HG, 128), 0)
    dl = lane - 2 * sub

    def row_bcast(p, r):
        return [jnp.broadcast_to(p[r:r + 1, 128 * i:128 * (i + 1)], (HG, 128)) for i in range(NC)]

    def pv_block(j, hh, r, pb):
        acc = []
        for half in range(2):
            alo = ahi = None
            for i in range(4 * half, 4 * half + 4):
                w = v32[j, i, hh, pl.ds(8 * r, 8), :]
                lo = _lo(w) * pb[i]
                hi = _hi(w) * pb[i]
                alo = lo if alo is None else alo + lo
                ahi = hi if ahi is None else ahi + hi
            acc.append((alo, ahi))
        rlo = jnp.sum(acc[0][0], axis=-1, keepdims=True) + jnp.sum(acc[1][0], axis=-1, keepdims=True)
        rhi = jnp.sum(acc[0][1], axis=-1, keepdims=True) + jnp.sum(acc[1][1], axis=-1, keepdims=True)
        return rlo, rhi

    def attention1(x, b):
        h = _ln(x).astype(bf16)

        def aligned(i):
            return i if isinstance(i, int) else pl.multiple_of(i, 8)

        def last_part(j, g, p, pb, rl):
            t0 = NT - 3
            out = None
            for t in (t0 + 1, t0, t0 + 2):
                if t == t0 + 1:
                    o = None
                    for c in range(NC):
                        vrows = jnp.concatenate([v32[j, c, HG - 2, pl.ds(64, 32), :],
                                                 v32[j, c, HG - 1, pl.ds(0, 32), :]], axis=0)
                        d = jax.lax.dot_general(pb[:, 128 * c:128 * (c + 1)], _as_bf16(vrows),
                                                (((1,), (1,)), ((), ())), preferred_element_type=f32)
                        o = d if o is None else o + d
                    tile = jnp.where(mask[:, 128 * t:128 * (t + 1)], o * rl, 0.0)
                else:
                    hh = (128 * t) // DH
                    pbs = row_bcast(p, hh)
                    tile = jnp.zeros((HG, 128), f32)
                    for c in range(128 * t, 128 * t + 128, 16):
                        rlo, rhi = pv_block(j, hh, (c % DH) // 16, pbs)
                        tile = jnp.where(dl == c % 128, rlo, jnp.where(dl == c % 128 + 1, rhi, tile))
                    tile = tile * jnp.broadcast_to(rl[hh:hh + 1, :], (HG, 128))
                d = wo_proj(tile.astype(bf16), g * (GW // 2) + 64 * t, 64)
                out = d if out is None else out + d
            return out

        def group(g, acc):
            j = b * NG + g
            q = jnp.concatenate(
                [_mm(h, _as_bf16(wq32[g * NT + t])) for t in range(NT)], axis=1)
            qbd = jnp.where(mask, q, 0.0).astype(bf16)
            wait_all(kbuf.at[j], ksem.at[g])

            @when(g == 3)
            def _():
                start_k(j + 1)
            s = jnp.concatenate(
                [_mm(qbd, _as_bf16(k32[j, c].reshape(HG * DH2, 128))) for c in range(NC)],
                axis=1) * SCALE
            m = jnp.max(s, axis=-1, keepdims=True)
            p = jnp.exp(s - m)
            l = jnp.sum(p, axis=-1, keepdims=True)
            pb = p.astype(bf16)
            rl = 1.0 / l
            for part in range(HG // VP):
                wait_all(vbuf.at[j, :, pl.ds(part * VP, VP)], vsem.at[(g % 2) * (HG // VP) + part])
                if part == HG // VP - 1:
                    @when(g == 3)
                    def _():
                        start_v(j + 1)
                if isinstance(g, int) and part == HG // VP - 1:
                    acc = acc + last_part(j, g, p, pb, rl)
                    break
                o = None
                for c in range(NC):
                    d = jax.lax.dot_general(
                        pb[:, 128 * c:128 * (c + 1)],
                        _as_bf16(v32[j, c, pl.ds(part * VP, VP)].reshape(VP * DH2, 128)),
                        (((1,), (1,)), ((), ())), preferred_element_type=f32)
                    o = d if o is None else o + d
                cols = slice(part * VP * DH, (part + 1) * VP * DH)
                om = jnp.where(mask[:, cols], o * rl, 0.0).astype(bf16)
                acc = acc + wo_proj(om, aligned(g * (GW // 2) + part * VP * DH2), VP * DH2)

            @when((g % 2) == 0)
            def _():
                start_v(j + 2 - g // 2)

            @when(g == 1)
            def _():
                start_k(j + 2)
            return acc

        acc = jnp.zeros((HG, D), f32)
        if isinstance(b, int):
            acc = group(NG - 1, jax.lax.fori_loop(0, NG - 1, group, acc))
        else:
            acc = jax.lax.fori_loop(0, NG, group, acc)
        return x + jnp.broadcast_to(jnp.sum(acc, axis=0, keepdims=True), (HG, D))

    def spread(v, rblk):
        t, base = divmod(16 * rblk, 128)
        vt = v[:, 128 * t:128 * (t + 1)]
        even = jnp.sum(jnp.where(dl == base, vt, 0.0), axis=-1, keepdims=True)
        odd = jnp.sum(jnp.where(dl == base + 1, vt, 0.0), axis=-1, keepdims=True)
        return even, odd

    def rowsum(a):
        return jnp.broadcast_to(jnp.sum(a, axis=0, keepdims=True), a.shape)

    def attention2(x, b, feed):
        h = _ln(x).astype(bf16)
        st = {'acc': None}
        N = NG * NT

        def tile_mask(t):
            c = lane + 128 * t
            return (c >= sub * DH) & (c < sub * DH + DH)

        def vpu_q():
            hr = h.astype(f32)
            acc = {}
            for rb in range(D // 16):
                even, odd = spread(hr, rb)
                if 'gate' in st:
                    even = even + st['gate']
                for u in range(N - VQ, N):
                    w = wq32[u, pl.ds(8 * rb, 8), :]
                    d = _lo(w) * even + _hi(w) * odd
                    acc[u] = d if rb == 0 else acc[u] + d
                yield
            for u in range(N - VQ, N):
                st['q', u] = jnp.where(tile_mask(u % UT), rowsum(acc[u]), 0.0).astype(bf16)

        vq = vpu_q()

        def q_tile(u):
            if u >= N - VQ:
                return
            for _ in range(VQP):
                next(vq, None)
            q = _mm(h, _as_bf16(wq32[u]))
            st['gate'] = q * 0.0
            st['q', u] = jnp.where(tile_mask(u % UT), q, 0.0).astype(bf16)

        def k_rows(c, u):
            hd, r0 = divmod(64 * u, DH2)
            g, h0 = divmod(hd, HG)
            j = b * NG + g
            if r0 + 64 <= DH2:
                return k32[j, c, h0, pl.ds(r0, 64), :]
            return jnp.concatenate([k32[j, c, h0, pl.ds(r0, DH2 - r0), :],
                                    k32[j, c, h0 + 1, pl.ds(0, 64 - (DH2 - r0)), :]], axis=0)

        def s_tile(u):
            k, t = divmod(u, UT)
            qt = st.pop(('q', u))
            d = jnp.concatenate([_mm(qt, _as_bf16(k_rows(c, u))) for c in range(NC)], axis=1)
            st['s', k] = d if t == 0 else st['s', k] + d
            if t == UT - 1:
                sa = st.pop(('s', k))
                m = jnp.max(sa, axis=-1, keepdims=True)
                p = jnp.exp2((sa - m) * (SCALE * LOG2E))
                st['p', k] = p
                st['rl', k] = 1.0 / jnp.sum(p, axis=-1, keepdims=True)

        def fac(hd):
            if ('f', hd) not in st:
                st['f', hd] = jnp.broadcast_to(st['rl', hd // U][hd % U:hd % U + 1, :], (HG, 128))
            return st['f', hd]

        def v_tile(u):
            p = st['p', u // UT]
            tile = jnp.zeros((HG, 128), f32)
            for c in range(128 * u, 128 * u + 128, 16):
                hd, r = c // DH, (c % DH) // 16
                g, hh = divmod(hd, HG)
                if ('pb', hd) not in st:
                    st['pb', hd] = row_bcast(p, hd % U)
                rlo, rhi = pv_block(b * NG + g, hh, r, st['pb', hd])
                if u >= VWO:
                    rlo = (rlo * fac(hd)).astype(bf16).astype(f32)
                    rhi = (rhi * fac(hd)).astype(bf16).astype(f32)
                    for n in range(ND):
                        w = wo32[n, pl.ds(c // 2, 8), :]
                        d = _lo(w) * rlo + _hi(w) * rhi
                        st['vacc', n] = st['vacc', n] + d if ('vacc', n) in st else d
                else:
                    base = c % 128
                    tile = jnp.where(dl == base, rlo, jnp.where(dl == base + 1, rhi, tile))
            if u < VWO:
                ha, hb = (128 * u) // DH, (128 * u + 127) // DH
                f = fac(ha) if ha == hb else jnp.where(lane < hb * DH - 128 * u, fac(ha), fac(hb))
                st['t', u] = (tile * f).astype(bf16)

        def w_tile(u):
            if u >= VWO:
                return
            d = wo_proj(st.pop(('t', u)), 64 * u, 64)
            st['acc'] = d if st['acc'] is None else st['acc'] + d

        SL = SLEAD * UT
        for m in range(-SL - QLEAD, N + WLAG):
            if m == MFEED:
                feed()
            if 0 <= m + SL + QLEAD < N:
                q_tile(m + SL + QLEAD)
            if 0 <= m + SL < N:
                s_tile(m + SL)
            if 0 <= m < N:
                v_tile(m)
            if 0 <= m - WLAG < N:
                w_tile(m - WLAG)
        for _ in vq:
            pass
        acc = st['acc'] + jnp.concatenate([st['vacc', n] for n in range(ND)], axis=1)
        return x + jnp.broadcast_to(jnp.sum(acc, axis=0, keepdims=True), (HG, D))

    def ffn(x):
        h = _ln(x)
        r = jnp.sum(h * wr_row, axis=-1, keepdims=True)
        hb = h.astype(bf16)
        a = [None] * NF
        accs = {}
        gate = [None]

        def act(g, u):
            return (g * jax.nn.sigmoid(g) * u).astype(bf16)

        def vpu_blocks():
            hr = hb.astype(f32)
            for rb in range(D // 16):
                even, odd = spread(hr, rb)
                if gate[0] is not None:
                    even = even + gate[0]
                for t in range(NF - NV, NF):
                    for nm, w32 in (('g', wg32), ('u', wu32)):
                        w = w32[t, pl.ds(8 * rb, 8), :]
                        d = _lo(w) * even + _hi(w) * odd
                        accs[nm, t] = d if rb == 0 else accs[nm, t] + d
                yield

        blocks = vpu_blocks()
        per = -(-(D // 16) // (NF - NV))
        for t in range(NF - NV):
            for _ in range(per):
                next(blocks, None)
            g = _mm(hb, _as_bf16(wg32[t]))
            u = _mm(hb, _as_bf16(wu32[t]))
            gate[0] = g * 0.0
            a[t] = act(g, u)
        for _ in blocks:
            pass
        for t in range(NF - NV, NF):
            a[t] = act(rowsum(accs['g', t]), rowsum(accs['u', t]))
        nk = NF - DV
        am = jnp.concatenate(a[:nk], axis=1)
        y = [_mm(am, _as_bf16(wd32[n, pl.ds(0, 64 * nk), :])) for n in range(ND)]
        yv = [None] * ND
        for t in range(nk, NF):
            af = a[t].astype(f32)
            for rb in range(8):
                even, odd = spread(af, rb)
                for n in range(ND):
                    w = wd32[n, pl.ds(64 * t + 8 * rb, 8), :]
                    d = _lo(w) * even + _hi(w) * odd
                    yv[n] = d if yv[n] is None else yv[n] + d
        y = jnp.concatenate([y[n] + rowsum(yv[n]) for n in range(ND)], axis=1)
        return x + h + y * jax.nn.sigmoid(r)

    def batch(b, out):
        xb = jnp.sum(jnp.where(row4 == b, x_all, 0.0), axis=0, keepdims=True)
        x = jnp.broadcast_to(xb, (HG, D))
        x = attention1(x, b)
        x = ffn(x)
        start_k(b * NG + 5)
        x = attention2(x, b, lambda: start_v(b * NG + 5))
        start_k(b * NG + 6)
        x = ffn(x)
        return jnp.where(row4 == b, x[:B, :], out)

    out = jax.lax.fori_loop(0, B - 1, batch, jnp.zeros((B, D), f32))
    out = batch(B - 1, out)
    o_ref[...] = out.astype(o_ref.dtype)


@jax.jit
def pallas_interleave_layers__sliding_block_cached__moe_arch_mod__decode_kernel(
    A_x: jax.Array,
    A_k_cache: jax.Array,
    A_v_cache: jax.Array,
    A_wq: jax.Array,
    A_wo: jax.Array,
    B_x: jax.Array,
    B_w_r: jax.Array,
    B_w_gate: jax.Array,
    B_w_up: jax.Array,
    B_w_down: jax.Array,
):
    del B_x
    k_t = jnp.transpose(A_k_cache, (0, 1, 3, 2))
    v_t = jnp.transpose(A_v_cache, (0, 1, 3, 2))
    any_spec = pl.BlockSpec(memory_space=pl.ANY)
    out = pl.pallas_call(
        _kernel,
        out_shape=jax.ShapeDtypeStruct((B, D), A_x.dtype),
        in_specs=[any_spec] * 9,
        out_specs=pl.BlockSpec(memory_space=pltpu.VMEM),
        scratch_shapes=[
            pltpu.VMEM((NJ, NC, HG, DH, 128), bf16),
            pltpu.VMEM((NJ, NC, HG, DH, 128), bf16),
            pltpu.VMEM((H * DH // 128, D, 128), bf16),
            pltpu.VMEM((ND, H * DH, 128), bf16),
            pltpu.VMEM((NF, D, 128), bf16),
            pltpu.VMEM((NF, D, 128), bf16),
            pltpu.VMEM((ND, F, 128), bf16),
            pltpu.VMEM((B, D), bf16),
            pltpu.VMEM((ND, 128), bf16),
            pltpu.SemaphoreType.DMA((NG,)),
            pltpu.SemaphoreType.DMA((2 * HG // VP,)),
            pltpu.SemaphoreType.DMA(()),
        ],
        compiler_params=pltpu.CompilerParams(vmem_limit_bytes=126 * 1024 * 1024),
    )(A_x.reshape(B, D), B_w_r.reshape(ND, 128), k_t, v_t,
      A_wq, A_wo, B_w_gate, B_w_up, B_w_down)
    return out.reshape(B, 1, D)
```
